```python
import jax
import jax.numpy as jnp

def _softmax(x, axis=-1):
    return jax.nn.softmax(x, axis=axis)
def _gelu(x):
    return jax.nn.gelu(x, approximate=True)
def _silu(x):
    return jax.nn.silu(x)
def _sigmoid(x):
    return jax.nn.sigmoid(x)
def _layernorm(x, axis=-1, eps=1e-5):
    m = jnp.mean(x, axis=axis, keepdims=True)
    v = jnp.var(x, axis=axis, keepdims=True)
    return (x - m) / jnp.sqrt(v + eps)
def _scatter_add(tgt, idx, src, axis=0):
    return tgt.at[idx].add(src)
def _segment_sum(src, seg, n):
    return jax.ops.segment_sum(src, seg, n)
class _Rng:
    def __init__(self, key):
        self._k = key
    def _next(self):
        self._k, sub = jax.random.split(self._k)
        return sub
    def normal(self, shape):
        return jax.random.normal(self._next(), shape, dtype=jnp.bfloat16)
    def randint(self, lo, hi, shape):
        return jax.random.randint(self._next(), shape, lo, hi, dtype=jnp.int32)
    def uniform(self, shape, lo=0.0, hi=1.0):
        return jax.random.uniform(self._next(), shape, jnp.bfloat16, lo, hi)
    def permutation(self, n):
        return jax.random.permutation(self._next(), n)


kernel_name = 'sequential_preLN__sliding_block_cached__moe_arch_mod__decode'

def setup_inputs():
    _rng = _Rng(jax.random.key(int.from_bytes(__import__("os").urandom(4), "little")))
    _w = (lambda a: (lambda t: t.astype(jnp.bfloat16) if jnp.issubdtype(t.dtype, jnp.floating) else t)(jnp.asarray(a)))
    def _A_setup():
        B, Sq, D = 1, 1, 640
        Hq, Hkv, Sk, Dh = 32, 32, 32768, 192
        assert Hq % Hkv == 0, (Hq, Hkv)
        return {
            "x": _w((lambda *s: _rng.normal(s) * 0.05)(B, Sq, D)),
            "k_cache": _w((lambda *s: _rng.normal(s) * 0.05)(B, Hkv, Sk, Dh)),
            "v_cache": _w((lambda *s: _rng.normal(s) * 0.05)(B, Hkv, Sk, Dh)),
            "wq": _w((lambda *s: _rng.normal(s) * 0.05)(D, Hq * Dh) * (D ** -0.5)),
            "wo": _w((lambda *s: _rng.normal(s) * 0.05)(Hq * Dh, D) * ((Hq * Dh) ** -0.5)),
        }
    _A_in = _A_setup()

    def _B_setup():
        B, S, D, F, C = 1, 1, 640, 1536, 1
        return {
            "x": _w((lambda *s: _rng.normal(s) * 0.05)(B, S, D)),
            "w_r": _w((lambda *s: _rng.normal(s) * 0.05)(D)),
            "w_gate": _w((lambda *s: _rng.normal(s) * 0.05)(D, F)),
            "w_up": _w((lambda *s: _rng.normal(s) * 0.05)(D, F)),
            "w_down": _w((lambda *s: _rng.normal(s) * 0.05)(F, D)),
        }
    _B_in = _B_setup()

    return {
        "A_x": _A_in["x"],
        "A_k_cache": _A_in["k_cache"],
        "A_v_cache": _A_in["v_cache"],
        "A_wq": _A_in["wq"],
        "A_wo": _A_in["wo"],
        "B_x": _B_in["x"],
        "B_w_r": _B_in["w_r"],
        "B_w_gate": _B_in["w_gate"],
        "B_w_up": _B_in["w_up"],
        "B_w_down": _B_in["w_down"],
    }

def reference(A_x, A_k_cache, A_v_cache, A_wq, A_wo, B_x, B_w_r, B_w_gate, B_w_up, B_w_down):
    def _A_ref(x, k_cache, v_cache, wq, wo):
        B, Sq, D = x.shape
        Hq, Dh = 32, 192
        Hkv, Sk = k_cache.shape[1], k_cache.shape[2]
        W = min(4096, max(256, Sk // 4))
        rep = Hq // Hkv
        q = (lambda x, *d: x.transpose(*d))((x @ wq).reshape(B, Sq, Hq, Dh), 0, 2, 1, 3)
        k = jnp.repeat(k_cache[:, :, Sk - W:, :], rep, axis=1)
        v = jnp.repeat(v_cache[:, :, Sk - W:, :], rep, axis=1)
        scores = jnp.einsum("bhqd,bhkd->bhqk", q, k) * (Dh ** -0.5)
        p = _softmax(scores, axis=-1)
        o = jnp.einsum("bhqk,bhkd->bhqd", p, v)
        return (lambda x, *d: x.transpose(*d))(o, 0, 2, 1, 3).reshape(B, Sq, Hq * Dh) @ wo

    def _B_ref(x, w_r, w_gate, w_up, w_down):
        B, S, D = x.shape
        C = 1
        r = x @ w_r
        idx = jnp.argsort(-r, axis=-1)[:, :C]
        idx_e = jnp.repeat(idx.reshape(B, C, 1), D, axis=2)
        x_sel = jnp.take_along_axis(x, idx_e, axis=1)
        g = _silu(x_sel @ w_gate)
        u = x_sel @ w_up
        y = (g * u) @ w_down
        r_sel = _sigmoid(jnp.take_along_axis(r, idx, axis=1))
        y = y * r_sel.reshape(B, C, 1)
        b_off = (jnp.arange(B) * S).reshape(B, 1)
        flat_idx = (idx + b_off).reshape(B * C)
        zero = (x * 0.0).reshape(B * S, D)
        upd = _scatter_add(zero, flat_idx, y.reshape(B * C, D), axis=0)
        return x + upd.reshape(B, S, D)

    x = A_x
    h = x + _A_ref(_layernorm(x, axis=-1), A_k_cache, A_v_cache, A_wq, A_wo)
    h2 = h + _B_ref(_layernorm(h, axis=-1), B_w_r, B_w_gate, B_w_up, B_w_down)
    return h2
```

```python
import functools

import jax
import jax.numpy as jnp
from jax import lax
import jax.experimental.pallas as pl
import jax.experimental.pallas.tpu as pltpu

_F32 = jnp.float32
_BF16 = jnp.bfloat16
_LN_EPS = 1e-5


def _layernorm(x):
    m = jnp.mean(x, axis=-1, keepdims=True)
    c = x - m
    v = jnp.mean(c * c, axis=-1, keepdims=True)
    return c / jnp.sqrt(v + _LN_EPS)


def _kernel(x_hbm, wr_hbm, k_hbm, v_hbm, wq_hbm, wo_hbm, wg_hbm, wu_hbm, wd_hbm,
            o_ref,
            x_buf, wr_buf, kbuf, vbuf, wq_buf, wo_buf, wg_buf, wu_buf, wd_buf,
            q_scr, sem_small, sem_wq, sem_k, sem_v, sem_wo, sem_g, sem_u, sem_d,
            *, H, Dh, Sk, W, D, F, NB, WQ_CH, GU_CH, WD_CH):
    n_wq = D // WQ_CH
    n_gu = D // GU_CH
    n_wd = F // WD_CH

    def x_dma():
        return pltpu.make_async_copy(x_hbm, x_buf, sem_small.at[0])

    def wr_dma():
        return pltpu.make_async_copy(wr_hbm, wr_buf, sem_small.at[1])

    def wq_dma(c):
        return pltpu.make_async_copy(wq_hbm.at[pl.ds(c * WQ_CH, WQ_CH)],
                                     wq_buf.at[pl.ds(c * WQ_CH, WQ_CH)], sem_wq.at[c])

    def k_dma(h, slot):
        return pltpu.make_async_copy(k_hbm.at[h, :, pl.ds(Sk - W, W)], kbuf.at[slot], sem_k.at[slot])

    def v_dma(h, slot):
        return pltpu.make_async_copy(v_hbm.at[h, :, pl.ds(Sk - W, W)], vbuf.at[slot], sem_v.at[slot])

    def wo_dma(h, slot):
        return pltpu.make_async_copy(wo_hbm.at[h], wo_buf.at[slot], sem_wo.at[slot])

    def g_dma(c):
        return pltpu.make_async_copy(wg_hbm.at[pl.ds(c * GU_CH, GU_CH)],
                                     wg_buf.at[pl.ds(c * GU_CH, GU_CH)], sem_g.at[c])

    def u_dma(c):
        return pltpu.make_async_copy(wu_hbm.at[pl.ds(c * GU_CH, GU_CH)],
                                     wu_buf.at[pl.ds(c * GU_CH, GU_CH)], sem_u.at[c])

    def d_dma(c):
        return pltpu.make_async_copy(wd_hbm.at[pl.ds(c * WD_CH, WD_CH)],
                                     wd_buf.at[pl.ds(c * WD_CH, WD_CH)], sem_d.at[c])

    def start_head(h, slot):
        k_dma(h, slot).start()
        wo_dma(h, slot).start()
        v_dma(h, slot).start()

    def start_ffn():
        for c in range(n_gu):
            g_dma(c).start()
            u_dma(c).start()
        for c in range(n_wd):
            d_dma(c).start()

    x_dma().start()
    wr_dma().start()
    for c in range(n_wq):
        wq_dma(c).start()
    for s in range(NB):
        start_head(s, s)

    x_dma().wait()
    x = x_buf[...].astype(_F32)
    xn = _layernorm(x).astype(_BF16)
    q = jnp.zeros((1, H * Dh), _F32)
    for c in range(n_wq):
        wq_dma(c).wait()
        q = q + jnp.dot(xn[:, c * WQ_CH:(c + 1) * WQ_CH], wq_buf[pl.ds(c * WQ_CH, WQ_CH), :],
                        preferred_element_type=_F32)
    q = q.astype(_BF16)
    for h in range(H):
        q_scr[h, :, :] = q[:, h * Dh:(h + 1) * Dh]

    scale = Dh ** -0.5

    def head_body(h, acc):
        slot = h % NB
        k_dma(h, slot).wait()
        qh = q_scr[h]
        s = jnp.dot(qh, kbuf[slot], preferred_element_type=_F32) * scale
        m = jnp.max(s, axis=-1, keepdims=True)
        p = jnp.exp(s - m)
        l = jnp.sum(p, axis=-1, keepdims=True)
        v_dma(h, slot).wait()
        o = lax.dot_general(p.astype(_BF16), vbuf[slot], (((1,), (1,)), ((), ())),
                            preferred_element_type=_F32)
        o = (o / l).astype(_BF16)
        wo_dma(h, slot).wait()
        acc = acc + jnp.dot(o, wo_buf[slot], preferred_element_type=_F32)

        @pl.when(h + NB < H)
        def _():
            start_head(h + NB, slot)

        @pl.when(h + NB == H)
        def _():
            start_ffn()

        return acc

    attn = lax.fori_loop(0, H, head_body, jnp.zeros((1, D), _F32))

    hres = x + attn
    hn = _layernorm(hres)
    hb = hn.astype(_BF16)
    wr_dma().wait()
    r = jnp.sum(hb.astype(_F32) * wr_buf[...].astype(_F32), axis=-1, keepdims=True)
    gate = jax.nn.sigmoid(r)
    g = jnp.zeros((1, F), _F32)
    u = jnp.zeros((1, F), _F32)
    for c in range(n_gu):
        hc = hb[:, c * GU_CH:(c + 1) * GU_CH]
        g_dma(c).wait()
        g = g + jnp.dot(hc, wg_buf[pl.ds(c * GU_CH, GU_CH), :], preferred_element_type=_F32)
        u_dma(c).wait()
        u = u + jnp.dot(hc, wu_buf[pl.ds(c * GU_CH, GU_CH), :], preferred_element_type=_F32)
    a = (g * jax.nn.sigmoid(g) * u).astype(_BF16)
    y = jnp.zeros((1, D), _F32)
    for c in range(n_wd):
        d_dma(c).wait()
        y = y + jnp.dot(a[:, c * WD_CH:(c + 1) * WD_CH], wd_buf[pl.ds(c * WD_CH, WD_CH), :],
                        preferred_element_type=_F32)
    upd = hn * 0.0 + y * gate
    o_ref[...] = (hres + (hn + upd)).astype(o_ref.dtype)


@jax.jit
def pallas_sequential_preLN__sliding_block_cached__moe_arch_mod__decode_kernel(
    A_x: jax.Array,
    A_k_cache: jax.Array,
    A_v_cache: jax.Array,
    A_wq: jax.Array,
    A_wo: jax.Array,
    B_x: jax.Array,
    B_w_r: jax.Array,
    B_w_gate: jax.Array,
    B_w_up: jax.Array,
    B_w_down: jax.Array,
):
    B, Sq, D = A_x.shape
    _, H, Sk, Dh = A_k_cache.shape
    F = B_w_gate.shape[1]
    W = min(4096, max(256, Sk // 4))
    NB = 4
    WQ_CH, GU_CH, WD_CH = 128, 128, 256

    kt = jnp.swapaxes(A_k_cache, 2, 3).reshape(H, Dh, Sk)
    vt = jnp.swapaxes(A_v_cache, 2, 3).reshape(H, Dh, Sk)
    x2 = A_x.reshape(1, D)
    wr2 = B_w_r.reshape(1, D)
    wo3 = A_wo.reshape(H, Dh, D)

    kern = functools.partial(_kernel, H=H, Dh=Dh, Sk=Sk, W=W, D=D, F=F, NB=NB,
                             WQ_CH=WQ_CH, GU_CH=GU_CH, WD_CH=WD_CH)
    any_spec = pl.BlockSpec(memory_space=pl.ANY)
    out = pl.pallas_call(
        kern,
        out_shape=jax.ShapeDtypeStruct((1, D), A_x.dtype),
        in_specs=[any_spec] * 9,
        out_specs=pl.BlockSpec(memory_space=pltpu.VMEM),
        scratch_shapes=[
            pltpu.VMEM((1, D), _BF16),
            pltpu.VMEM((1, D), _BF16),
            pltpu.VMEM((NB, Dh, W), _BF16),
            pltpu.VMEM((NB, Dh, W), _BF16),
            pltpu.VMEM((D, H * Dh), _BF16),
            pltpu.VMEM((NB, Dh, D), _BF16),
            pltpu.VMEM((D, F), _BF16),
            pltpu.VMEM((D, F), _BF16),
            pltpu.VMEM((F, D), _BF16),
            pltpu.VMEM((H, 1, Dh), _BF16),
            pltpu.SemaphoreType.DMA((2,)),
            pltpu.SemaphoreType.DMA((D // WQ_CH,)),
            pltpu.SemaphoreType.DMA((NB,)),
            pltpu.SemaphoreType.DMA((NB,)),
            pltpu.SemaphoreType.DMA((NB,)),
            pltpu.SemaphoreType.DMA((D // GU_CH,)),
            pltpu.SemaphoreType.DMA((D // GU_CH,)),
            pltpu.SemaphoreType.DMA((F // WD_CH,)),
        ],
        compiler_params=pltpu.CompilerParams(vmem_limit_bytes=100 * 1024 * 1024),
    )(x2, wr2, kt, vt, A_wq, wo3, B_w_gate, B_w_up, B_w_down)
    return out.reshape(B, Sq, D)
```

```python
import contextlib
import functools

import jax
import jax.numpy as jnp
from jax import lax
import jax.experimental.pallas as pl
import jax.experimental.pallas.tpu as pltpu

_F32 = jnp.float32
_BF16 = jnp.bfloat16
_LN_EPS = 1e-5
_LANES = 128


def _layernorm(x):
    m = jnp.mean(x, axis=-1, keepdims=True)
    c = x - m
    v = jnp.mean(c * c, axis=-1, keepdims=True)
    return c / jnp.sqrt(v + _LN_EPS)


def _chunks(sizes):
    out, o = [], 0
    for s in sizes:
        out.append((o, s))
        o += s
    return out


def _kernel(x_hbm, wr_hbm, k_hbm, v_hbm, wq_hbm, wo_hbm, wg_hbm, wu_hbm, wd_hbm,
            o_ref,
            x_buf, wr_buf, kbuf, vbuf, wq_buf, wo_buf, wg_buf, wu_buf, wd_buf,
            q_scr, sem_small, sem_wq, sem_k, sem_v, sem_wo, sem_g, sem_u, sem_d,
            *, H, Dh, Sk, W, D, F, NB, WQ, GU, WD, PK, PV, PWO, PW, PF, SCOPES):
    scope = jax.named_scope if SCOPES else (lambda name: contextlib.nullcontext())
    wq_c, gu_c, wd_c = _chunks(WQ), _chunks(GU), _chunks(WD)

    def x_dma():
        return pltpu.make_async_copy(x_hbm, x_buf, sem_small.at[0])

    def wr_dma():
        return pltpu.make_async_copy(wr_hbm, wr_buf, sem_small.at[1])

    def row_dma(src, dst, sem, cs, c):
        o, s = cs[c]
        return pltpu.make_async_copy(src.at[pl.ds(o, s)], dst.at[pl.ds(o, s)], sem.at[c])

    wq_dma = lambda c: row_dma(wq_hbm, wq_buf, sem_wq, wq_c, c)
    g_dma = lambda c: row_dma(wg_hbm, wg_buf, sem_g, gu_c, c)
    u_dma = lambda c: row_dma(wu_hbm, wu_buf, sem_u, gu_c, c)
    d_dma = lambda c: row_dma(wd_hbm, wd_buf, sem_d, wd_c, c)

    def k_dma(h, slot):
        return pltpu.make_async_copy(k_hbm.at[h, :, pl.ds(Sk - W, W)], kbuf.at[slot], sem_k.at[slot])

    def v_dma(h, slot):
        return pltpu.make_async_copy(v_hbm.at[h, :, pl.ds(Sk - W, W)], vbuf.at[slot], sem_v.at[slot])

    def wo_dma(h, slot):
        return pltpu.make_async_copy(wo_hbm.at[h], wo_buf.at[slot], sem_wo.at[slot])

    def start_head(h, slot):
        k_dma(h, slot).start(priority=PK)
        wo_dma(h, slot).start(priority=PWO)
        v_dma(h, slot).start(priority=PV)

    ffn_dmas = ([functools.partial(g_dma, c) for c in range(len(gu_c))]
                + [functools.partial(u_dma, c) for c in range(len(gu_c))]
                + [functools.partial(d_dma, c) for c in range(len(wd_c))])
    n_in_loop = min(NB, len(ffn_dmas))

    x_dma().start()
    wr_dma().start()
    for c in range(len(wq_c)):
        wq_dma(c).start(priority=PW)

    def prologue(s, carry):
        start_head(s, s)
        return carry

    lax.fori_loop(0, NB, prologue, 0)

    x_dma().wait()
    x = x_buf[...].astype(_F32)
    xn = _layernorm(x).astype(_BF16)
    q = None
    for c, (o, s) in enumerate(wq_c):
        with scope("wait_wq"):
            wq_dma(c).wait()
        with scope("qproj"):
            t = jnp.dot(xn[:, o:o + s], wq_buf[pl.ds(o, s), :], preferred_element_type=_F32)
            q = t if q is None else q + t
    with scope("qstore"):
        q = q.astype(_BF16)
        for h in range(H):
            q_scr[h, :, :] = q[:, h * Dh:(h + 1) * Dh]

    scale = Dh ** -0.5

    def head_body(h, acc):
        slot = h % NB
        with scope("wait_k"):
            k_dma(h, slot).wait()
        with scope("qk"):
            qh = q_scr[h]
            s = jnp.dot(qh, kbuf[slot], preferred_element_type=_F32) * scale
            m = jnp.max(s, axis=-1, keepdims=True)
            p = jnp.exp(s - m)
            l = jnp.sum(p, axis=-1, keepdims=True)
        with scope("wait_v"):
            v_dma(h, slot).wait()
        with scope("pv"):
            o = lax.dot_general(p.astype(_BF16), vbuf[slot], (((1,), (1,)), ((), ())),
                                preferred_element_type=_F32)
            o = (o / l).astype(_BF16)
        with scope("wait_wo"):
            wo_dma(h, slot).wait()
        with scope("wo"):
            acc = acc + jnp.dot(o, wo_buf[slot], preferred_element_type=_F32)

        @pl.when(h + NB < H)
        def _():
            start_head(h + NB, slot)

        for i in range(n_in_loop):
            @pl.when(h + NB == H + i)
            def _(i=i):
                ffn_dmas[i]().start(priority=PF)

        return acc

    attn = lax.fori_loop(0, H, head_body, jnp.zeros((1, D), _F32))
    for d in ffn_dmas[n_in_loop:]:
        d().start(priority=PF)

    hres = x + attn
    hn = _layernorm(hres)
    hb = hn.astype(_BF16)
    wr_dma().wait()
    hf = hb.astype(_F32)
    rv = None
    for c in range(D // _LANES):
        t = hf[:, c * _LANES:(c + 1) * _LANES] * wr_buf[c:c + 1, :].astype(_F32)
        rv = t if rv is None else rv + t
    r = jnp.sum(rv, axis=-1, keepdims=True)
    gate = jax.nn.sigmoid(r)
    g = None
    for c, (o, s) in enumerate(gu_c):
        with scope("wait_g"):
            g_dma(c).wait()
        with scope("gate"):
            t = jnp.dot(hb[:, o:o + s], wg_buf[pl.ds(o, s), :], preferred_element_type=_F32)
            g = t if g is None else g + t
    g = g * jax.nn.sigmoid(g)
    u = None
    for c, (o, s) in enumerate(gu_c):
        with scope("wait_u"):
            u_dma(c).wait()
        with scope("up"):
            t = jnp.dot(hb[:, o:o + s], wu_buf[pl.ds(o, s), :], preferred_element_type=_F32)
            u = t if u is None else u + t
    a = (g * u).astype(_BF16)
    base = hres + (hn + hn * 0.0)
    y = None
    for c, (o, s) in enumerate(wd_c):
        with scope("wait_d"):
            d_dma(c).wait()
        with scope("down"):
            t = jnp.dot(a[:, o:o + s], wd_buf[pl.ds(o, s), :], preferred_element_type=_F32)
            y = t if y is None else y + t
    with scope("final"):
        o_ref[...] = (base + y * gate).astype(o_ref.dtype)


def _build(NB=2, WQ=(640,), GU=(640,), WD=(1024, 384, 128), PK=0, PV=1, PWO=1, PW=1, PF=1, SCOPES=False):
    def fn(A_x, A_k_cache, A_v_cache, A_wq, A_wo, B_x, B_w_r, B_w_gate, B_w_up, B_w_down):
        B, Sq, D = A_x.shape
        _, H, Sk, Dh = A_k_cache.shape
        F = B_w_gate.shape[1]
        W = min(4096, max(256, Sk // 4))

        kt = jnp.swapaxes(A_k_cache, 2, 3).reshape(H, Dh, Sk)
        vt = jnp.swapaxes(A_v_cache, 2, 3).reshape(H, Dh, Sk)
        x2 = A_x.reshape(1, D)
        wr2 = B_w_r.reshape(D // _LANES, _LANES)
        wo3 = A_wo.reshape(H, Dh, D)

        kern = functools.partial(_kernel, H=H, Dh=Dh, Sk=Sk, W=W, D=D, F=F, NB=NB,
                                 WQ=WQ, GU=GU, WD=WD, PK=PK, PV=PV, PWO=PWO, PW=PW, PF=PF, SCOPES=SCOPES)
        any_spec = pl.BlockSpec(memory_space=pl.ANY)
        out = pl.pallas_call(
            kern,
            out_shape=jax.ShapeDtypeStruct((1, D), A_x.dtype),
            in_specs=[any_spec] * 9,
            out_specs=pl.BlockSpec(memory_space=pltpu.VMEM),
            scratch_shapes=[
                pltpu.VMEM((1, D), _BF16),
                pltpu.VMEM((D // _LANES, _LANES), _BF16),
                pltpu.VMEM((NB, Dh, W), _BF16),
                pltpu.VMEM((NB, Dh, W), _BF16),
                pltpu.VMEM((D, H * Dh), _BF16),
                pltpu.VMEM((NB, Dh, D), _BF16),
                pltpu.VMEM((D, F), _BF16),
                pltpu.VMEM((D, F), _BF16),
                pltpu.VMEM((F, D), _BF16),
                pltpu.VMEM((H, 1, Dh), _BF16),
                pltpu.SemaphoreType.DMA((2,)),
                pltpu.SemaphoreType.DMA((len(WQ),)),
                pltpu.SemaphoreType.DMA((NB,)),
                pltpu.SemaphoreType.DMA((NB,)),
                pltpu.SemaphoreType.DMA((NB,)),
                pltpu.SemaphoreType.DMA((len(GU),)),
                pltpu.SemaphoreType.DMA((len(GU),)),
                pltpu.SemaphoreType.DMA((len(WD),)),
            ],
            compiler_params=pltpu.CompilerParams(vmem_limit_bytes=100 * 1024 * 1024),
        )(x2, wr2, kt, vt, A_wq, wo3, B_w_gate, B_w_up, B_w_down)
        return out.reshape(B, Sq, D)
    return fn


@jax.jit
def pallas_sequential_preLN__sliding_block_cached__moe_arch_mod__decode_kernel(
    A_x: jax.Array,
    A_k_cache: jax.Array,
    A_v_cache: jax.Array,
    A_wq: jax.Array,
    A_wo: jax.Array,
    B_x: jax.Array,
    B_w_r: jax.Array,
    B_w_gate: jax.Array,
    B_w_up: jax.Array,
    B_w_down: jax.Array,
):
    return _build()(A_x, A_k_cache, A_v_cache, A_wq, A_wo, B_x, B_w_r, B_w_gate, B_w_up, B_w_down)
```

```python
import contextlib
import functools

import jax
import jax.numpy as jnp
from jax import lax
import jax.experimental.pallas as pl
import jax.experimental.pallas.tpu as pltpu

_F32 = jnp.float32
_BF16 = jnp.bfloat16
_LN_EPS = 1e-5
_LANES = 128


def _layernorm(x):
    m = jnp.mean(x, axis=-1, keepdims=True)
    c = x - m
    v = jnp.mean(c * c, axis=-1, keepdims=True)
    return c / jnp.sqrt(v + _LN_EPS)


def _log2(n):
    assert n > 0 and n & (n - 1) == 0, n
    return n.bit_length() - 1


def _div(x, n):
    return x >> _log2(n) if isinstance(x, int) else lax.shift_right_logical(x, _log2(n))


def _mod(x, n):
    assert n & (n - 1) == 0
    return x & (n - 1)


def _chunks(sizes):
    out, o = [], 0
    for s in sizes:
        out.append((o, s))
        o += s
    return out


def _kernel(x_hbm, wr_hbm, k_hbm, v_hbm, wq_hbm, wo_hbm, wg_hbm, wu_hbm, wd_hbm,
            o_ref,
            x_buf, wr_buf, kbuf, vbuf, wq_buf, wo_buf, wg_buf, wu_buf, wd_buf,
            q_scr, s_scr, p_scr, l_scr, oacc_scr, acc_scr,
            sem_small, sem_a, sem_b, sem_wq, sem_wo, sem_u, sem_d,
            *, H, Dh, Sk, W, D, F, KC, KA, VA, VP, NP, WQ_A, WU_A, WD, SCOPES):
    scope = jax.named_scope if SCOPES else (lambda name: contextlib.nullcontext())
    fscope = jax.named_scope if SCOPES == 2 else (lambda name: contextlib.nullcontext())
    wd_c = _chunks(WD)
    C = W // KC
    CP = C // NP
    PW = W // NP
    NSA = 1 << KA.bit_length()
    NSB = 1 << max(VA, VP).bit_length()
    LAG = C - CP // 2
    chunk_elems = Dh * KC
    wq_cw = chunk_elems // 8
    WQ_CS = (H * Dh) // wq_cw
    n_wq = (WQ_A // 8) * WQ_CS
    WG_R = chunk_elems // F
    wq_b = D - WQ_A
    wu_b = D - WU_A
    n_k = H * C
    n_g = D // WG_R
    n_f = n_g + WU_A // WG_R
    PA, PB = 0, 1

    def a_wq(i):
        rows = pl.ds(pl.multiple_of(wq_b + _div(i, WQ_CS) * 8, 8), 8)
        cols = pl.ds(pl.multiple_of(_mod(i, WQ_CS) * wq_cw, _LANES), wq_cw)
        return pltpu.make_async_copy(wq_hbm.at[rows, cols], wq_buf.at[rows, cols], sem_a.at[_mod(i, NSA)])

    def kv_chunk(src, dst, s, sem):
        h, c = _div(s, C), _mod(s, C)
        return pltpu.make_async_copy(
            src.at[h, :, pl.ds(pl.multiple_of(Sk - W + c * KC, KC), KC)],
            dst.at[_mod(h, 2), :, pl.ds(pl.multiple_of(c * KC, KC), KC)], sem)

    def a_k(s):
        return kv_chunk(k_hbm, kbuf, s, sem_a.at[_mod(s + n_wq, NSA)])

    def a_g(i):
        rows = pl.ds(pl.multiple_of(i * WG_R, WG_R), WG_R)
        return pltpu.make_async_copy(wg_hbm.at[rows], wg_buf.at[rows], sem_a.at[_mod(i + n_wq + n_k, NSA)])

    def a_u(i):
        rows = pl.ds(pl.multiple_of(wu_b + (i - n_g) * WG_R, WG_R), WG_R)
        return pltpu.make_async_copy(wu_hbm.at[rows], wu_buf.at[rows], sem_a.at[_mod(i + n_wq + n_k, NSA)])

    def start_f(i):
        @pl.when(i < n_g)
        def _():
            a_g(i).start(priority=PA)

        if n_f > n_g:
            @pl.when(jnp.logical_and(i >= n_g, i < n_f))
            def _():
                a_u(i).start(priority=PA)

    def x_dma():
        return pltpu.make_async_copy(x_hbm, x_buf, sem_small.at[0])

    def wr_dma():
        return pltpu.make_async_copy(wr_hbm, wr_buf, sem_small.at[1])

    def wq_dma():
        return pltpu.make_async_copy(wq_hbm.at[pl.ds(0, wq_b)], wq_buf.at[pl.ds(0, wq_b)], sem_wq.at[0])

    def b_v(s):
        return kv_chunk(v_hbm, vbuf, s, sem_b.at[_mod(s, NSB)])

    def wo_dma(h):
        return pltpu.make_async_copy(wo_hbm.at[h], wo_buf.at[_mod(h, 2)], sem_wo.at[_mod(h, 2)])

    def u_dma():
        return pltpu.make_async_copy(wu_hbm.at[pl.ds(0, wu_b)], wu_buf.at[pl.ds(0, wu_b)], sem_u.at[0])

    def d_dma(c):
        o, s = wd_c[c]
        return pltpu.make_async_copy(wd_hbm.at[pl.ds(o, s)], wd_buf.at[pl.ds(o, s)], sem_d.at[c])

    tail_dmas = [u_dma] + [functools.partial(d_dma, c) for c in range(len(wd_c))]

    x_dma().start(priority=PA)
    wr_dma().start(priority=PA)
    wq_dma().start(priority=PB)

    def first_a(i, carry):
        a_wq(i).start(priority=PA)
        return carry

    lax.fori_loop(0, KA, first_a, 0)

    def first_v(s, carry):
        b_v(s).start(priority=PB)
        return carry

    lax.fori_loop(0, VP, first_v, 0)
    wo_dma(0).start(priority=PB)

    x_dma().wait()
    x = x_buf[...].astype(_F32)
    xn = _layernorm(x).astype(_BF16)

    def pump_wq(i, carry):
        a_wq(i).wait()

        @pl.when(i + KA < n_wq)
        def _():
            a_wq(i + KA).start(priority=PA)

        @pl.when(i + KA >= n_wq)
        def _():
            a_k(i + KA - n_wq).start(priority=PA)

        return carry

    with scope("pump_wq"):
        lax.fori_loop(0, n_wq, pump_wq, 0)
    with scope("wait_wq"):
        wq_dma().wait()
    with scope("qproj"):
        q = jnp.dot(xn, wq_buf[...], preferred_element_type=_F32).astype(_BF16)
        for h in range(H):
            q_scr[h, :, :] = q[:, h * Dh:(h + 1) * Dh]
        acc_scr[...] = jnp.zeros(acc_scr.shape, _F32)
        oacc_scr[...] = jnp.zeros(oacc_scr.shape, _F32)

    scale = Dh ** -0.5

    def pv_piece(h, j):
        cols = pl.ds(pl.multiple_of(j * PW, PW), PW)
        oacc_scr[...] += lax.dot_general(p_scr[:, cols], vbuf[_mod(h, 2), :, cols], (((1,), (1,)), ((), ())),
                                         preferred_element_type=_F32)

    def head_out(h):
        o = (oacc_scr[...] / l_scr[...]).astype(_BF16)
        wo_dma(h).wait()
        return jnp.dot(o, wo_buf[_mod(h, 2)], preferred_element_type=_F32)

    def step(s, carry):
        h, c = _div(s, C), _mod(s, C)
        sv = s - LAG

        @pl.when(sv >= 0)
        def _():
            with fscope("wait_v"):
                b_v(sv).wait()

        @pl.when(s + KA < n_k)
        def _():
            a_k(s + KA).start(priority=PA)

        @pl.when(s + KA >= n_k)
        def _():
            start_f(s + KA - n_k)

        iv = sv + VA

        @pl.when(jnp.logical_and(iv >= VP, iv < n_k))
        def _():
            b_v(iv).start(priority=PB)

        for i, d in enumerate(tail_dmas):
            @pl.when(iv == n_k + i)
            def _(d=d):
                d().start(priority=PB)

        with fscope("wait_k"):
            a_k(s).wait()

        @pl.when(jnp.logical_and(c == 0, h > 0))
        def _():
            wo_dma(h).start(priority=PB)

        @pl.when(jnp.logical_and(_mod(c, CP) == CP // 2 - 1, h > 0))
        def _():
            with fscope("pv"):
                pv_piece(h - 1, _div(c, CP))

        @pl.when(jnp.logical_and(c == C - 2, h > 0))
        def _():
            with fscope("finish"):
                acc_scr[...] += head_out(h - 1)
                oacc_scr[...] = jnp.zeros(oacc_scr.shape, _F32)

        @pl.when(_mod(c, CP) == CP - 1)
        def _():
            with fscope("qk"):
                cols = pl.ds(pl.multiple_of(_div(c, CP) * PW, PW), PW)
                s_scr[:, cols] = jnp.dot(q_scr[h], kbuf[_mod(h, 2), :, cols],
                                         preferred_element_type=_F32) * scale

        @pl.when(c == C - 1)
        def _():
            with fscope("softmax"):
                sc = s_scr[...]
                m = jnp.max(sc, axis=-1, keepdims=True)
                p = jnp.exp(sc - m)
                l_scr[...] = jnp.sum(p, axis=-1, keepdims=True)
                p_scr[...] = p.astype(_BF16)

        return carry

    with scope("main"):
        lax.fori_loop(0, n_k, step, 0)

    def pump_f(i, carry):
        @pl.when(i < LAG)
        def _():
            b_v(n_k - LAG + i).wait()

        start_f(i + KA)

        @pl.when(i < n_g)
        def _():
            a_g(i).wait()

        if n_f > n_g:
            @pl.when(i >= n_g)
            def _():
                a_u(i).wait()

        @pl.when(jnp.logical_and(_mod(i, CP) == CP // 2 - 1, i < LAG))
        def _():
            pv_piece(H - 1, _div(i, CP))

        return carry

    assert n_f >= LAG and VA - LAG >= len(tail_dmas)
    with scope("pump_f"):
        lax.fori_loop(0, n_f, pump_f, 0)

    with scope("last_head"):
        attn = acc_scr[...] + head_out(H - 1)

    with scope("gate"):
        hres = x + attn
        hn = _layernorm(hres)
        hb = hn.astype(_BF16)
        wr_dma().wait()
        hf = hb.astype(_F32)
        rv = None
        for c in range(D // _LANES):
            t = hf[:, c * _LANES:(c + 1) * _LANES] * wr_buf[c:c + 1, :].astype(_F32)
            rv = t if rv is None else rv + t
        r = jnp.sum(rv, axis=-1, keepdims=True)
        gate = jax.nn.sigmoid(r)
        g = jnp.dot(hb, wg_buf[...], preferred_element_type=_F32)
        g = g * jax.nn.sigmoid(g)
    with scope("wait_u"):
        u_dma().wait()
    with scope("up"):
        u = jnp.dot(hb, wu_buf[...], preferred_element_type=_F32)
        a = (g * u).astype(_BF16)
        base = hres + (hn + hn * 0.0)
    y = None
    for c, (o, s) in enumerate(wd_c):
        with scope("wait_d"):
            d_dma(c).wait()
        with scope("down"):
            t = jnp.dot(a[:, o:o + s], wd_buf[pl.ds(o, s), :], preferred_element_type=_F32)
            y = t if y is None else y + t
    with scope("final"):
        o_ref[...] = (base + y * gate).astype(o_ref.dtype)


def _build(KC=128, KA=12, VA=48, VP=32, NP=4, WQ_A=320, WU_A=0, WD=(768, 512, 256), SKIPB=False, SCOPES=False):
    def fn(A_x, A_k_cache, A_v_cache, A_wq, A_wo, B_x, B_w_r, B_w_gate, B_w_up, B_w_down):
        B, Sq, D = A_x.shape
        _, H, Sk, Dh = A_k_cache.shape
        F = B_w_gate.shape[1]
        W = min(4096, max(256, Sk // 4))

        kt = jnp.swapaxes(A_k_cache, 2, 3).reshape(H, Dh, Sk)
        vt = jnp.swapaxes(A_v_cache, 2, 3).reshape(H, Dh, Sk)
        x2 = A_x.reshape(1, D)
        wr2 = B_w_r.reshape(D // _LANES, _LANES)
        wo3 = A_wo.reshape(H, Dh, D)

        kern = functools.partial(_kernel, H=H, Dh=Dh, Sk=Sk, W=W, D=D, F=F, KC=KC, KA=KA, VA=VA, VP=VP, NP=NP,
                                 WQ_A=WQ_A, WU_A=WU_A, WD=WD, SCOPES=SCOPES)
        any_spec = pl.BlockSpec(memory_space=pl.ANY)
        out = pl.pallas_call(
            kern,
            out_shape=jax.ShapeDtypeStruct((1, D), A_x.dtype),
            in_specs=[any_spec] * 9,
            out_specs=pl.BlockSpec(memory_space=pltpu.VMEM),
            scratch_shapes=[
                pltpu.VMEM((1, D), _BF16),
                pltpu.VMEM((D // _LANES, _LANES), _BF16),
                pltpu.VMEM((2, Dh, W), _BF16),
                pltpu.VMEM((2, Dh, W), _BF16),
                pltpu.VMEM((D, H * Dh), _BF16),
                pltpu.VMEM((2, Dh, D), _BF16),
                pltpu.VMEM((D, F), _BF16),
                pltpu.VMEM((D, F), _BF16),
                pltpu.VMEM((F, D), _BF16),
                pltpu.VMEM((H, 1, Dh), _BF16),
                pltpu.VMEM((1, W), _F32),
                pltpu.VMEM((1, W), _BF16),
                pltpu.VMEM((1, 1), _F32),
                pltpu.VMEM((1, Dh), _F32),
                pltpu.VMEM((1, D), _F32),
                pltpu.SemaphoreType.DMA((2,)),
                pltpu.SemaphoreType.DMA((1 << KA.bit_length(),)),
                pltpu.SemaphoreType.DMA((1 << max(VA, VP).bit_length(),)),
                pltpu.SemaphoreType.DMA((1,)),
                pltpu.SemaphoreType.DMA((2,)),
                pltpu.SemaphoreType.DMA((1,)),
                pltpu.SemaphoreType.DMA((len(WD),)),
            ],
            compiler_params=pltpu.CompilerParams(vmem_limit_bytes=100 * 1024 * 1024,
                                                 disable_bounds_checks=True,
                                                 disable_semaphore_checks=True,
                                                 skip_device_barrier=SKIPB),
        )(x2, wr2, kt, vt, A_wq, wo3, B_w_gate, B_w_up, B_w_down)
        return out.reshape(B, Sq, D)
    return fn


@jax.jit
def pallas_sequential_preLN__sliding_block_cached__moe_arch_mod__decode_kernel(
    A_x: jax.Array,
    A_k_cache: jax.Array,
    A_v_cache: jax.Array,
    A_wq: jax.Array,
    A_wo: jax.Array,
    B_x: jax.Array,
    B_w_r: jax.Array,
    B_w_gate: jax.Array,
    B_w_up: jax.Array,
    B_w_down: jax.Array,
):
    return _build()(A_x, A_k_cache, A_v_cache, A_wq, A_wo, B_x, B_w_r, B_w_gate, B_w_up, B_w_down)
```

```python
import contextlib
import functools

import jax
import jax.numpy as jnp
from jax import lax
import jax.experimental.pallas as pl
import jax.experimental.pallas.tpu as pltpu

_F32 = jnp.float32
_BF16 = jnp.bfloat16
_LN_EPS = 1e-5
_LANES = 128


def _layernorm(x):
    m = jnp.mean(x, axis=-1, keepdims=True)
    c = x - m
    v = jnp.mean(c * c, axis=-1, keepdims=True)
    return c / jnp.sqrt(v + _LN_EPS)


def _log2(n):
    assert n > 0 and n & (n - 1) == 0, n
    return n.bit_length() - 1


def _div(x, n):
    return x >> _log2(n) if isinstance(x, int) else lax.shift_right_logical(x, _log2(n))


def _mod(x, n):
    assert n & (n - 1) == 0
    return x & (n - 1)


def _kernel(x_hbm, wr_hbm, k_hbm, v_hbm, wq_hbm, wo_hbm, wg_hbm, wu_hbm, wd_hbm,
            o_ref,
            x_buf, wr_buf, kbuf, vbuf, wq_buf, wo_buf, wg_buf, wu_buf, wd_buf,
            xn_scr, q_scr, s_scr, p_scr, l_scr, oacc_scr, acc_scr,
            hb_scr, base_scr, gate_scr, g_scr, u_scr,
            sem_small, sem_a, sem_b, sem_wo,
            *, H, Dh, Sk, W, D, F, KA, VA, NP, UA, WDR, DOWN, SKIP, SCOPES):
    scope = jax.named_scope if SCOPES else (lambda name: contextlib.nullcontext())
    KC = _LANES
    C = W // KC
    CP = C // NP
    PW = W // NP
    NSA = 1 << KA.bit_length()
    NSB = 1 << VA.bit_length()
    LAG = C - CP // 2
    QC = Dh * KC // 8
    QS = (H * Dh) // QC
    n_q = (D // 8) * QS
    n_qa = (n_q - LAG) // 2
    n_qb = n_q - n_qa
    assert n_qb - n_qa == LAG and n_qa % QS == 0
    GR = Dh * KC // F
    n_kv = H * C
    n_g = D // GR
    UB = n_g - UA
    n_d = F // WDR
    PA, PB = 0, 1

    a_k0, a_g0, a_u0, a_end = n_qa, n_qa + n_kv, n_qa + n_kv + n_g, n_qa + n_kv + n_g + UA
    b_v0, b_u0, b_d0, b_end = n_qb, n_qb + n_kv, n_qb + n_kv + UB, n_qb + n_kv + UB + n_d

    def wq_chunk(i, first_row, sem):
        rows = pl.ds(pl.multiple_of(first_row + _div(i, QS) * 8, 8), 8)
        cols = pl.ds(pl.multiple_of(_mod(i, QS) * QC, _LANES), QC)
        return pltpu.make_async_copy(wq_hbm.at[rows, cols], wq_buf.at[rows, cols], sem)

    def kv_chunk(src, dst, s, sem):
        h, c = _div(s, C), _mod(s, C)
        return pltpu.make_async_copy(
            src.at[h, :, pl.ds(pl.multiple_of(Sk - W + c * KC, KC), KC)],
            dst.at[_mod(h, 2), :, pl.ds(pl.multiple_of(c * KC, KC), KC)], sem)

    def row_chunk(src, dst, first_row, nrows, sem):
        rows = pl.ds(pl.multiple_of(first_row, nrows), nrows)
        return pltpu.make_async_copy(src.at[rows], dst.at[rows], sem)

    def a_desc(kind, a):
        sem = sem_a.at[_mod(a, NSA)]
        if kind == "q":
            return wq_chunk(a, (n_qb // QS) * 8, sem)
        if kind == "k":
            return kv_chunk(k_hbm, kbuf, a - a_k0, sem)
        if kind == "g":
            return row_chunk(wg_hbm, wg_buf, (a - a_g0) * GR, GR, sem)
        return row_chunk(wu_hbm, wu_buf, (UB + a - a_u0) * GR, GR, sem)

    def b_desc(kind, b):
        sem = sem_b.at[_mod(b, NSB)]
        if kind == "q":
            return wq_chunk(b, 0, sem)
        if kind == "v":
            return kv_chunk(v_hbm, vbuf, b - b_v0, sem)
        if kind == "u":
            return row_chunk(wu_hbm, wu_buf, (b - b_u0) * GR, GR, sem)
        return row_chunk(wd_hbm, wd_buf, (b - b_d0) * WDR, WDR, sem)

    a_range = {"q": (0, a_k0), "k": (a_k0, a_g0), "g": (a_g0, a_u0), "u": (a_u0, a_end)}
    b_range = {"q": (0, b_v0), "v": (b_v0, b_u0), "u": (b_u0, b_d0), "d": (b_d0, b_end)}

    def dispatch(desc, ranges, idx, lo, hi, action):
        for kind, (k_lo, k_hi) in ranges.items():
            if k_hi <= lo or k_lo >= hi or k_lo == k_hi:
                continue
            conds = []
            if k_lo > lo:
                conds.append(idx >= k_lo)
            if k_hi < hi:
                conds.append(idx < k_hi)
            if not conds:
                action(desc(kind, idx))
            else:
                cond = conds[0] if len(conds) == 1 else jnp.logical_and(conds[0], conds[1])
                pl.when(cond)(functools.partial(lambda kind: action(desc(kind, idx)), kind))

    def pump(t, lo, hi):
        dispatch(b_desc, b_range, t + LAG_B, lo + LAG_B, hi + LAG_B, lambda d: d.wait())
        dispatch(a_desc, a_range, t + KA, lo + KA, hi + KA, lambda d: d.start(priority=PA))
        dispatch(b_desc, b_range, t + LAG_B + VA, lo + LAG_B + VA, hi + LAG_B + VA,
                 lambda d: d.start(priority=PB))
        dispatch(a_desc, a_range, t, lo, hi, lambda d: d.wait())

    LAG_B = 0

    def x_dma():
        return pltpu.make_async_copy(x_hbm, x_buf, sem_small.at[0])

    def wr_dma():
        return pltpu.make_async_copy(wr_hbm, wr_buf, sem_small.at[1])

    def wo_dma(h):
        return pltpu.make_async_copy(wo_hbm.at[h], wo_buf.at[_mod(h, 2)], sem_wo.at[_mod(h, 2)])

    x_dma().start(priority=PA)
    wr_dma().start(priority=PA)

    def first(i, carry):
        @pl.when(i < KA)
        def _():
            a_desc("q", i).start(priority=PA)

        b_desc("q", i).start(priority=PB)
        return carry

    assert KA <= VA <= n_qb and KA <= n_qa
    lax.fori_loop(0, VA, first, 0)

    x_dma().wait()
    x = x_buf[...].astype(_F32)
    xn_scr[...] = _layernorm(x).astype(_BF16)
    acc_scr[...] = jnp.zeros(acc_scr.shape, _F32)
    oacc_scr[...] = jnp.zeros(oacc_scr.shape, _F32)

    scale = Dh ** -0.5

    def q_pair(p):
        cols = pl.ds(pl.multiple_of(p * (2 * Dh), _LANES), 2 * Dh)
        q2 = jnp.dot(xn_scr[...], wq_buf[:, cols], preferred_element_type=_F32).astype(_BF16)
        q_scr[2 * p] = q2[:, :Dh]
        q_scr[2 * p + 1] = q2[:, Dh:]

    def softmax():
        sc = s_scr[...]
        m = jnp.max(sc, axis=-1, keepdims=True)
        p = jnp.exp(sc - m)
        l_scr[...] = jnp.sum(p, axis=-1, keepdims=True)
        p_scr[...] = p.astype(_BF16)

    def pv_piece(h, j):
        cols = pl.ds(pl.multiple_of(j * PW, PW), PW)
        oacc_scr[...] += lax.dot_general(p_scr[:, cols], vbuf[_mod(h, 2), :, cols], (((1,), (1,)), ((), ())),
                                         preferred_element_type=_F32)

    def head_out(h):
        o = (oacc_scr[...] / l_scr[...]).astype(_BF16)
        wo_dma(h).wait()
        return jnp.dot(o, wo_buf[_mod(h, 2)], preferred_element_type=_F32)

    t1 = a_k0 + C

    def phase1(t, carry):
        pump(t, 0, t1)

        @pl.when(t == a_k0)
        def _():
            wo_dma(0).start(priority=PB)

        return carry

    with scope("phase1"):
        lax.fori_loop(0, t1, phase1, 0)
    assert t1 >= n_qb
    with scope("head0"):
        q_pair(0)
        s_scr[...] = jnp.dot(q_scr[0], kbuf[0], preferred_element_type=_F32) * scale
        softmax()

    def phase2(lo, hi, t, carry):
        s = t - a_k0
        h, c = _div(s, C), _mod(s, C)
        pump(t, lo, hi)

        @pl.when(c == 0)
        def _():
            wo_dma(h).start(priority=PB)

        @pl.when(_mod(c, CP) == CP // 2 - 1)
        def _():
            if "pv" not in SKIP:
                pv_piece(h - 1, _div(c, CP))

        @pl.when(c == C - 2)
        def _():
            acc_scr[...] += head_out(h - 1)
            oacc_scr[...] = jnp.zeros(oacc_scr.shape, _F32)

        @pl.when(jnp.logical_and(jnp.logical_and(c == CP + CP // 2 + 1, _mod(h, 2) == 1), h + 1 < H))
        def _():
            q_pair(_div(h + 1, 2))

        @pl.when(_mod(c, CP) == CP - 1)
        def _():
            if "qk" not in SKIP:
                cols = pl.ds(pl.multiple_of(_div(c, CP) * PW, PW), PW)
                s_scr[:, cols] = jnp.dot(q_scr[h], kbuf[_mod(h, 2), :, cols],
                                         preferred_element_type=_F32) * scale

        @pl.when(c == C - 1)
        def _():
            softmax()

        return carry

    t2 = a_g0
    t2m = min(a_g0 - KA, b_u0 - VA)
    with scope("phase2"):
        lax.fori_loop(t1, t2m, functools.partial(phase2, t1, t2m), 0)
        lax.fori_loop(t2m, t2, functools.partial(phase2, t2m, t2), 0)

    t3 = a_end
    u_b_rows = UB * GR
    UA1 = UA - _LANES // GR
    u_mid = u_b_rows + UA1 * GR

    def phase3(t, carry):
        pump(t, t2, t3)
        tau = t - t2

        @pl.when(jnp.logical_and(_mod(tau, CP) == CP // 2 - 1, tau < LAG))
        def _():
            pv_piece(H - 1, _div(tau, CP))

        @pl.when(tau == LAG)
        def _():
            hres = x_buf[...].astype(_F32) + acc_scr[...] + head_out(H - 1)
            hn = _layernorm(hres)
            hb = hn.astype(_BF16)
            wr_dma().wait()
            hf = hb.astype(_F32)
            rv = None
            for c in range(D // _LANES):
                tt = hf[:, c * _LANES:(c + 1) * _LANES] * wr_buf[c:c + 1, :].astype(_F32)
                rv = tt if rv is None else rv + tt
            r = jnp.sum(rv, axis=-1, keepdims=True)
            gate_scr[...] = jax.nn.sigmoid(r)
            hb_scr[...] = hb
            base_scr[...] = hres + (hn + hn * 0.0)

        @pl.when(tau == n_g)
        def _():
            g = jnp.dot(hb_scr[...], wg_buf[...], preferred_element_type=_F32)
            g_scr[...] = g * jax.nn.sigmoid(g)

        @pl.when(tau == max(LAG + UB, n_g) + 1)
        def _():
            u_scr[...] = jnp.dot(hb_scr[:, :u_b_rows], wu_buf[pl.ds(0, u_b_rows), :],
                                 preferred_element_type=_F32)

        @pl.when(tau == max(n_g + UA1, max(LAG + UB, n_g) + 2))
        def _():
            u_scr[...] += jnp.dot(hb_scr[:, u_b_rows:u_mid], wu_buf[pl.ds(u_b_rows, u_mid - u_b_rows), :],
                                  preferred_element_type=_F32)

        return carry

    assert LAG < n_g and max(n_g + UA1, max(LAG + UB, n_g) + 2) < t3 - t2
    with scope("phase3"):
        lax.fori_loop(t2, t3, phase3, 0)

    with scope("up"):
        u = u_scr[...] + jnp.dot(hb_scr[:, u_mid:], wu_buf[pl.ds(u_mid, D - u_mid), :],
                                 preferred_element_type=_F32)
        a = (g_scr[...] * u).astype(_BF16)

    def wait_d(b, carry):
        b_desc("d", b).wait()
        return carry

    y = None
    row = 0
    done = t3
    assert done >= b_d0 and sum(DOWN) == F
    for rows in DOWN:
        need = b_d0 + (row + rows) // WDR
        if need > done:
            with scope("wait_d"):
                lax.fori_loop(done, need, wait_d, 0)
            done = need
        with scope("down"):
            tt = jnp.dot(a[:, row:row + rows], wd_buf[pl.ds(row, rows), :], preferred_element_type=_F32)
            y = tt if y is None else y + tt
        row += rows
    assert done == b_end
    with scope("final"):
        o_ref[...] = (base_scr[...] + y * gate_scr[...]).astype(o_ref.dtype)


def _build(KA=12, VA=48, NP=4, UA=24, WDR=32, DOWN=(640, 384, 256, 128, 128), SKIP=(), SCOPES=False,
           INTERPRET=False):
    def fn(A_x, A_k_cache, A_v_cache, A_wq, A_wo, B_x, B_w_r, B_w_gate, B_w_up, B_w_down):
        B, Sq, D = A_x.shape
        _, H, Sk, Dh = A_k_cache.shape
        F = B_w_gate.shape[1]
        W = min(4096, max(256, Sk // 4))

        kt = jnp.swapaxes(A_k_cache, 2, 3).reshape(H, Dh, Sk)
        vt = jnp.swapaxes(A_v_cache, 2, 3).reshape(H, Dh, Sk)
        x2 = A_x.reshape(1, D)
        wr2 = B_w_r.reshape(D // _LANES, _LANES)
        wo3 = A_wo.reshape(H, Dh, D)

        kern = functools.partial(_kernel, H=H, Dh=Dh, Sk=Sk, W=W, D=D, F=F, KA=KA, VA=VA, NP=NP,
                                 UA=UA, WDR=WDR, DOWN=DOWN, SKIP=SKIP, SCOPES=SCOPES)
        any_spec = pl.BlockSpec(memory_space=pl.ANY)
        out = pl.pallas_call(
            kern,
            out_shape=jax.ShapeDtypeStruct((1, D), A_x.dtype),
            in_specs=[any_spec] * 9,
            out_specs=pl.BlockSpec(memory_space=pltpu.VMEM),
            scratch_shapes=[
                pltpu.VMEM((1, D), _BF16),
                pltpu.VMEM((D // _LANES, _LANES), _BF16),
                pltpu.VMEM((2, Dh, W), _BF16),
                pltpu.VMEM((2, Dh, W), _BF16),
                pltpu.VMEM((D, H * Dh), _BF16),
                pltpu.VMEM((2, Dh, D), _BF16),
                pltpu.VMEM((D, F), _BF16),
                pltpu.VMEM((D, F), _BF16),
                pltpu.VMEM((F, D), _BF16),
                pltpu.VMEM((1, D), _BF16),
                pltpu.VMEM((H, 1, Dh), _BF16),
                pltpu.VMEM((1, W), _F32),
                pltpu.VMEM((1, W), _BF16),
                pltpu.VMEM((1, 1), _F32),
                pltpu.VMEM((1, Dh), _F32),
                pltpu.VMEM((1, D), _F32),
                pltpu.VMEM((1, D), _BF16),
                pltpu.VMEM((1, D), _F32),
                pltpu.VMEM((1, 1), _F32),
                pltpu.VMEM((1, F), _F32),
                pltpu.VMEM((1, F), _F32),
                pltpu.SemaphoreType.DMA((2,)),
                pltpu.SemaphoreType.DMA((1 << KA.bit_length(),)),
                pltpu.SemaphoreType.DMA((1 << VA.bit_length(),)),
                pltpu.SemaphoreType.DMA((2,)),
            ],
            compiler_params=pltpu.CompilerParams(vmem_limit_bytes=100 * 1024 * 1024,
                                                 disable_bounds_checks=True,
                                                 disable_semaphore_checks=True),
            interpret=INTERPRET,
        )(x2, wr2, kt, vt, A_wq, wo3, B_w_gate, B_w_up, B_w_down)
        return out.reshape(B, Sq, D)
    return fn


@jax.jit
def pallas_sequential_preLN__sliding_block_cached__moe_arch_mod__decode_kernel(
    A_x: jax.Array,
    A_k_cache: jax.Array,
    A_v_cache: jax.Array,
    A_wq: jax.Array,
    A_wo: jax.Array,
    B_x: jax.Array,
    B_w_r: jax.Array,
    B_w_gate: jax.Array,
    B_w_up: jax.Array,
    B_w_down: jax.Array,
):
    return _build()(A_x, A_k_cache, A_v_cache, A_wq, A_wo, B_x, B_w_r, B_w_gate, B_w_up, B_w_down)
```

```python
import contextlib
import functools

import jax
import jax.numpy as jnp
from jax import lax
import jax.experimental.pallas as pl
import jax.experimental.pallas.tpu as pltpu

_F32 = jnp.float32
_BF16 = jnp.bfloat16
_LN_EPS = 1e-5
_LANES = 128


def _layernorm(x):
    m = jnp.mean(x, axis=-1, keepdims=True)
    c = x - m
    v = jnp.mean(c * c, axis=-1, keepdims=True)
    return c / jnp.sqrt(v + _LN_EPS)


def _log2(n):
    assert n > 0 and n & (n - 1) == 0, n
    return n.bit_length() - 1


def _div(x, n):
    return x >> _log2(n) if isinstance(x, int) else lax.shift_right_logical(x, _log2(n))


def _mod(x, n):
    assert n & (n - 1) == 0
    return x & (n - 1)


def _kernel(x_hbm, wr_hbm, k_hbm, v_hbm, wq_hbm, wo_hbm, wg_hbm, wu_hbm, wd_hbm,
            o_ref,
            x_buf, wr_buf, kbuf, vbuf, wq_buf, wo_buf, wg_buf, wu_buf, wd_buf,
            xn_scr, q_scr, s_scr, p_scr, l_scr, oacc_scr, acc_scr,
            hb_scr, base_scr, gate_scr, g_scr, u_scr,
            sem_small, sem_a, sem_b, sem_wo,
            *, H, Dh, Sk, W, D, F, KA, VA, NP, UA, WDR, DOWN, QSH, WOR, WOS, SKIP, SCOPES):
    scope = jax.named_scope if SCOPES else (lambda name: contextlib.nullcontext())
    KC = _LANES
    C = W // KC
    CP = C // NP
    PW = W // NP
    NSA = 1 << KA.bit_length()
    NSB = 1 << VA.bit_length()
    LAG = C - CP // 2
    QR, QC = QSH
    nrb, ncb = D // QR, (H * Dh) // QC
    n_q = nrb * ncb
    n_qa = (n_q - LAG) // 2
    n_qb = n_q - n_qa
    assert n_qb - n_qa == LAG
    GR = Dh * KC // F
    n_kv = H * C
    n_g = D // GR
    UB = n_g - UA
    n_d = F // WDR
    PA, PB = 0, 1

    a_k0, a_g0, a_u0, a_end = n_qa, n_qa + n_kv, n_qa + n_kv + n_g, n_qa + n_kv + n_g + UA
    b_v0, b_u0, b_d0, b_end = n_qb, n_qb + n_kv, n_qb + n_kv + UB, n_qb + n_kv + UB + n_d

    def wq_chunk(i, sem):
        if ncb & (ncb - 1) == 0:
            rb, cb = _div(i, ncb), _mod(i, ncb)
        else:
            rb, cb = _mod(i, nrb), _div(i, nrb)
        rows = pl.ds(pl.multiple_of(rb * QR, QR), QR)
        cols = pl.ds(pl.multiple_of(cb * QC, _LANES), QC)
        return pltpu.make_async_copy(wq_hbm.at[rows, cols], wq_buf.at[rows, cols], sem)

    def kv_chunk(src, dst, s, sem):
        h, c = _div(s, C), _mod(s, C)
        return pltpu.make_async_copy(
            src.at[h, :, pl.ds(pl.multiple_of(Sk - W + c * KC, KC), KC)],
            dst.at[_mod(h, 2), :, pl.ds(pl.multiple_of(c * KC, KC), KC)], sem)

    def row_chunk(src, dst, first_row, nrows, sem):
        rows = pl.ds(pl.multiple_of(first_row, nrows), nrows)
        return pltpu.make_async_copy(src.at[rows], dst.at[rows], sem)

    def a_desc(kind, a):
        sem = sem_a.at[_mod(a, NSA)]
        if kind == "q":
            return wq_chunk(a + n_qb, sem)
        if kind == "k":
            return kv_chunk(k_hbm, kbuf, a - a_k0, sem)
        if kind == "g":
            return row_chunk(wg_hbm, wg_buf, (a - a_g0) * GR, GR, sem)
        return row_chunk(wu_hbm, wu_buf, (UB + a - a_u0) * GR, GR, sem)

    def b_desc(kind, b):
        sem = sem_b.at[_mod(b, NSB)]
        if kind == "q":
            return wq_chunk(b, sem)
        if kind == "v":
            return kv_chunk(v_hbm, vbuf, b - b_v0, sem)
        if kind == "u":
            return row_chunk(wu_hbm, wu_buf, (b - b_u0) * GR, GR, sem)
        return row_chunk(wd_hbm, wd_buf, (b - b_d0) * WDR, WDR, sem)

    a_range = {"q": (0, a_k0), "k": (a_k0, a_g0), "g": (a_g0, a_u0), "u": (a_u0, a_end)}
    b_range = {"q": (0, b_v0), "v": (b_v0, b_u0), "u": (b_u0, b_d0), "d": (b_d0, b_end)}

    def dispatch(desc, ranges, idx, lo, hi, action):
        for kind, (k_lo, k_hi) in ranges.items():
            if k_hi <= lo or k_lo >= hi or k_lo == k_hi:
                continue
            conds = []
            if k_lo > lo:
                conds.append(idx >= k_lo)
            if k_hi < hi:
                conds.append(idx < k_hi)
            if not conds:
                action(desc(kind, idx))
            else:
                cond = conds[0] if len(conds) == 1 else jnp.logical_and(conds[0], conds[1])
                pl.when(cond)(functools.partial(lambda kind: action(desc(kind, idx)), kind))

    def pump(t, lo, hi):
        dispatch(b_desc, b_range, t + LAG_B, lo + LAG_B, hi + LAG_B, lambda d: d.wait())
        dispatch(a_desc, a_range, t + KA, lo + KA, hi + KA, lambda d: d.start(priority=PA))
        dispatch(b_desc, b_range, t + LAG_B + VA, lo + LAG_B + VA, hi + LAG_B + VA,
                 lambda d: d.start(priority=PB))
        dispatch(a_desc, a_range, t, lo, hi, lambda d: d.wait())

    LAG_B = 0

    def x_dma():
        return pltpu.make_async_copy(x_hbm, x_buf, sem_small.at[0])

    def wr_dma():
        return pltpu.make_async_copy(wr_hbm, wr_buf, sem_small.at[1])

    def wo_dma(h):
        return pltpu.make_async_copy(wo_hbm.at[h], wo_buf.at[_mod(h, 2)], sem_wo.at[_mod(h, 2)])

    def wo_chunk(h, j):
        rows = pl.ds(pl.multiple_of(j * WOR, WOR), WOR)
        return pltpu.make_async_copy(wo_hbm.at[h, rows], wo_buf.at[_mod(h, 2), rows], sem_wo.at[_mod(h, 2)])

    def issue_wo(h, c):
        if not WOR:
            @pl.when(c == 0)
            def _():
                wo_dma(h).start(priority=PB)
            return
        nwo = Dh // WOR
        half = nwo // 2
        step = WOS
        off = min(2, step - 1)
        assert step * half <= C // 2

        @pl.when(jnp.logical_and(_mod(c, step) == off, c < step * half))
        def _():
            wo_chunk(h, 2 * _div(c, step)).start(priority=PB)

        @pl.when(jnp.logical_and(_mod(c, step) == off, jnp.logical_and(c >= C // 2, c < C // 2 + step * half)))
        def _():
            wo_chunk(h, 2 * _div(c - C // 2, step) + 1).start(priority=PA)

    x_dma().start(priority=PA)
    wr_dma().start(priority=PA)

    def first(i, carry):
        @pl.when(i < KA)
        def _():
            a_desc("q", i).start(priority=PA)

        b_desc("q", i).start(priority=PB)
        return carry

    assert KA <= VA <= n_qb and KA <= n_qa
    lax.fori_loop(0, VA, first, 0)

    x_dma().wait()
    x = x_buf[...].astype(_F32)
    xn_scr[...] = _layernorm(x).astype(_BF16)
    acc_scr[...] = jnp.zeros(acc_scr.shape, _F32)
    oacc_scr[...] = jnp.zeros(oacc_scr.shape, _F32)

    scale = Dh ** -0.5

    def q_pair(p):
        cols = pl.ds(pl.multiple_of(p * (2 * Dh), _LANES), 2 * Dh)
        q2 = jnp.dot(xn_scr[...], wq_buf[:, cols], preferred_element_type=_F32).astype(_BF16)
        q_scr[2 * p] = q2[:, :Dh]
        q_scr[2 * p + 1] = q2[:, Dh:]

    def softmax():
        sc = s_scr[...]
        m = jnp.max(sc, axis=-1, keepdims=True)
        p = jnp.exp(sc - m)
        l_scr[...] = jnp.sum(p, axis=-1, keepdims=True)
        p_scr[...] = p.astype(_BF16)

    def pv_piece(h, j):
        cols = pl.ds(pl.multiple_of(j * PW, PW), PW)
        oacc_scr[...] += lax.dot_general(p_scr[:, cols], vbuf[_mod(h, 2), :, cols], (((1,), (1,)), ((), ())),
                                         preferred_element_type=_F32)

    def head_out(h):
        o = (oacc_scr[...] / l_scr[...]).astype(_BF16)
        wo_dma(h).wait()
        return jnp.dot(o, wo_buf[_mod(h, 2)], preferred_element_type=_F32)

    t1 = a_k0 + C

    def phase1(t, carry):
        pump(t, 0, t1)

        @pl.when(t >= a_k0)
        def _():
            issue_wo(0, t - a_k0)

        return carry

    if SCOPES == 3:
        cuts = [0, 8, 16, 32, 48, 66, 82, 98]
        for lo_, hi_ in zip(cuts[:-1], cuts[1:]):
            with scope("p1_%d_%d" % (lo_, hi_)):
                lax.fori_loop(lo_, hi_, phase1, 0)
    else:
        with scope("phase1"):
            lax.fori_loop(0, t1, phase1, 0)
    assert t1 >= n_qb
    with scope("head0"):
        q_pair(0)
        s_scr[...] = jnp.dot(q_scr[0], kbuf[0], preferred_element_type=_F32) * scale
        softmax()

    def phase2(lo, hi, t, carry):
        s = t - a_k0
        h, c = _div(s, C), _mod(s, C)
        pump(t, lo, hi)

        issue_wo(h, c)

        @pl.when(_mod(c, CP) == CP // 2 - 1)
        def _():
            if "pv" not in SKIP:
                pv_piece(h - 1, _div(c, CP))

        @pl.when(c == C - 2)
        def _():
            acc_scr[...] += head_out(h - 1)
            oacc_scr[...] = jnp.zeros(oacc_scr.shape, _F32)

        @pl.when(jnp.logical_and(jnp.logical_and(c == CP + CP // 2 + 1, _mod(h, 2) == 1), h + 1 < H))
        def _():
            q_pair(_div(h + 1, 2))

        @pl.when(_mod(c, CP) == CP - 1)
        def _():
            if "qk" not in SKIP:
                cols = pl.ds(pl.multiple_of(_div(c, CP) * PW, PW), PW)
                s_scr[:, cols] = jnp.dot(q_scr[h], kbuf[_mod(h, 2), :, cols],
                                         preferred_element_type=_F32) * scale

        @pl.when(c == C - 1)
        def _():
            softmax()

        return carry

    t2 = a_g0
    t2m = min(a_g0 - KA, b_u0 - VA)
    with scope("phase2"):
        if SCOPES == 3:
            cuts = [t1, t1 + 32, t1 + 64, t1 + 128, t1 + 256, t1 + 512, t2m]
            for lo_, hi_ in zip(cuts[:-1], cuts[1:]):
                with scope("p2_%d_%d" % (lo_, hi_)):
                    lax.fori_loop(lo_, hi_, functools.partial(phase2, t1, t2m), 0)
        else:
            lax.fori_loop(t1, t2m, functools.partial(phase2, t1, t2m), 0)
        lax.fori_loop(t2m, t2, functools.partial(phase2, t2m, t2), 0)

    t3 = a_end
    u_b_rows = UB * GR
    UA1 = UA - _LANES // GR
    u_mid = u_b_rows + UA1 * GR

    def phase3(t, carry):
        pump(t, t2, t3)
        tau = t - t2

        @pl.when(jnp.logical_and(_mod(tau, CP) == CP // 2 - 1, tau < LAG))
        def _():
            pv_piece(H - 1, _div(tau, CP))

        @pl.when(tau == LAG)
        def _():
            hres = x_buf[...].astype(_F32) + acc_scr[...] + head_out(H - 1)
            hn = _layernorm(hres)
            hb = hn.astype(_BF16)
            wr_dma().wait()
            hf = hb.astype(_F32)
            rv = None
            for c in range(D // _LANES):
                tt = hf[:, c * _LANES:(c + 1) * _LANES] * wr_buf[c:c + 1, :].astype(_F32)
                rv = tt if rv is None else rv + tt
            r = jnp.sum(rv, axis=-1, keepdims=True)
            gate_scr[...] = jax.nn.sigmoid(r)
            hb_scr[...] = hb
            base_scr[...] = hres + (hn + hn * 0.0)

        @pl.when(tau == n_g)
        def _():
            g = jnp.dot(hb_scr[...], wg_buf[...], preferred_element_type=_F32)
            g_scr[...] = g * jax.nn.sigmoid(g)

        @pl.when(tau == max(LAG + UB, n_g) + 1)
        def _():
            u_scr[...] = jnp.dot(hb_scr[:, :u_b_rows], wu_buf[pl.ds(0, u_b_rows), :],
                                 preferred_element_type=_F32)

        @pl.when(tau == max(n_g + UA1, max(LAG + UB, n_g) + 2))
        def _():
            u_scr[...] += jnp.dot(hb_scr[:, u_b_rows:u_mid], wu_buf[pl.ds(u_b_rows, u_mid - u_b_rows), :],
                                  preferred_element_type=_F32)

        return carry

    assert LAG < n_g and max(n_g + UA1, max(LAG + UB, n_g) + 2) < t3 - t2
    with scope("phase3"):
        lax.fori_loop(t2, t3, phase3, 0)

    with scope("up"):
        u = u_scr[...] + jnp.dot(hb_scr[:, u_mid:], wu_buf[pl.ds(u_mid, D - u_mid), :],
                                 preferred_element_type=_F32)
        a = (g_scr[...] * u).astype(_BF16)

    def wait_d(b, carry):
        b_desc("d", b).wait()
        return carry

    y = None
    row = 0
    done = t3
    assert done >= b_d0 and sum(DOWN) == F
    for rows in DOWN:
        need = b_d0 + (row + rows) // WDR
        if need > done:
            with scope("wait_d"):
                lax.fori_loop(done, need, wait_d, 0)
            done = need
        with scope("down"):
            tt = jnp.dot(a[:, row:row + rows], wd_buf[pl.ds(row, rows), :], preferred_element_type=_F32)
            y = tt if y is None else y + tt
        row += rows
    assert done == b_end
    with scope("final"):
        o_ref[...] = (base_scr[...] + y * gate_scr[...]).astype(o_ref.dtype)


def _build(KA=12, VA=48, NP=4, UA=24, WDR=32, DOWN=(640, 384, 256, 128, 128), QSH=(8, 3072), WOR=24, WOS=1, SKIP=(), SCOPES=False,
           INTERPRET=False):
    def fn(A_x, A_k_cache, A_v_cache, A_wq, A_wo, B_x, B_w_r, B_w_gate, B_w_up, B_w_down):
        B, Sq, D = A_x.shape
        _, H, Sk, Dh = A_k_cache.shape
        F = B_w_gate.shape[1]
        W = min(4096, max(256, Sk // 4))

        kt = jnp.swapaxes(A_k_cache, 2, 3).reshape(H, Dh, Sk)
        vt = jnp.swapaxes(A_v_cache, 2, 3).reshape(H, Dh, Sk)
        x2 = A_x.reshape(1, D)
        wr2 = B_w_r.reshape(D // _LANES, _LANES)
        wo3 = A_wo.reshape(H, Dh, D)

        kern = functools.partial(_kernel, H=H, Dh=Dh, Sk=Sk, W=W, D=D, F=F, KA=KA, VA=VA, NP=NP,
                                 UA=UA, WDR=WDR, DOWN=DOWN, QSH=QSH, WOR=WOR, WOS=WOS, SKIP=SKIP, SCOPES=SCOPES)
        any_spec = pl.BlockSpec(memory_space=pl.ANY)
        out = pl.pallas_call(
            kern,
            out_shape=jax.ShapeDtypeStruct((1, D), A_x.dtype),
            in_specs=[any_spec] * 9,
            out_specs=pl.BlockSpec(memory_space=pltpu.VMEM),
            scratch_shapes=[
                pltpu.VMEM((1, D), _BF16),
                pltpu.VMEM((D // _LANES, _LANES), _BF16),
                pltpu.VMEM((2, Dh, W), _BF16),
                pltpu.VMEM((2, Dh, W), _BF16),
                pltpu.VMEM((D, H * Dh), _BF16),
                pltpu.VMEM((2, Dh, D), _BF16),
                pltpu.VMEM((D, F), _BF16),
                pltpu.VMEM((D, F), _BF16),
                pltpu.VMEM((F, D), _BF16),
                pltpu.VMEM((1, D), _BF16),
                pltpu.VMEM((H, 1, Dh), _BF16),
                pltpu.VMEM((1, W), _F32),
                pltpu.VMEM((1, W), _BF16),
                pltpu.VMEM((1, 1), _F32),
                pltpu.VMEM((1, Dh), _F32),
                pltpu.VMEM((1, D), _F32),
                pltpu.VMEM((1, D), _BF16),
                pltpu.VMEM((1, D), _F32),
                pltpu.VMEM((1, 1), _F32),
                pltpu.VMEM((1, F), _F32),
                pltpu.VMEM((1, F), _F32),
                pltpu.SemaphoreType.DMA((2,)),
                pltpu.SemaphoreType.DMA((1 << KA.bit_length(),)),
                pltpu.SemaphoreType.DMA((1 << VA.bit_length(),)),
                pltpu.SemaphoreType.DMA((2,)),
            ],
            compiler_params=pltpu.CompilerParams(vmem_limit_bytes=100 * 1024 * 1024,
                                                 disable_bounds_checks=True,
                                                 disable_semaphore_checks=True),
            interpret=INTERPRET,
        )(x2, wr2, kt, vt, A_wq, wo3, B_w_gate, B_w_up, B_w_down)
        return out.reshape(B, Sq, D)
    return fn


@jax.jit
def pallas_sequential_preLN__sliding_block_cached__moe_arch_mod__decode_kernel(
    A_x: jax.Array,
    A_k_cache: jax.Array,
    A_v_cache: jax.Array,
    A_wq: jax.Array,
    A_wo: jax.Array,
    B_x: jax.Array,
    B_w_r: jax.Array,
    B_w_gate: jax.Array,
    B_w_up: jax.Array,
    B_w_down: jax.Array,
):
    return _build()(A_x, A_k_cache, A_v_cache, A_wq, A_wo, B_x, B_w_r, B_w_gate, B_w_up, B_w_down)
```

```python
import functools

import jax
import jax.numpy as jnp
from jax import lax
import jax.experimental.pallas as pl
import jax.experimental.pallas.tpu as pltpu

_F32 = jnp.float32
_BF16 = jnp.bfloat16
_LN_EPS = 1e-5
_LANES = 128
_SUBLANES = 8


def _layernorm(x):
    m = jnp.mean(x, axis=-1, keepdims=True)
    c = x - m
    v = jnp.mean(c * c, axis=-1, keepdims=True)
    return c / jnp.sqrt(v + _LN_EPS)


def _log2(n):
    assert n > 0 and n & (n - 1) == 0, n
    return n.bit_length() - 1


def _div(x, n):
    return x >> _log2(n) if isinstance(x, int) else lax.shift_right_logical(x, _log2(n))


def _mod(x, n):
    assert n & (n - 1) == 0
    return x & (n - 1)


def _kernel(x_hbm, wr_hbm, k_hbm, v_hbm, wq_hbm, wo_hbm, wg_hbm, wu_hbm, wd_hbm,
            o_ref,
            x_buf, wr_buf, kbuf, vbuf, wq_buf, wo_buf, wg_buf, wu_buf, wd_buf,
            xn_scr, q_scr, s_scr, p_scr, l_scr, oacc_scr, acc_scr,
            hb_scr, base_scr, gate_scr, g_scr, u_scr,
            sem_small, sem_a, sem_b, sem_wo,
            *, H, Dh, Sk, W, D, F, KA, VA, NP, UA, WOR, WDR, DOWN):
    KC = _LANES
    C = W // KC
    CP = C // NP
    PW = W // NP
    NSA = 1 << KA.bit_length()
    NSB = 1 << VA.bit_length()
    LAG = C - CP // 2
    QC = Dh * KC // _SUBLANES
    QS = (H * Dh) // QC
    n_q = (D // _SUBLANES) * QS
    n_qa = (n_q - LAG) // 2
    n_qb = n_q - n_qa
    assert n_qb - n_qa == LAG
    GR = Dh * KC // F
    n_kv = H * C
    n_g = D // GR
    UB = n_g - UA
    n_d = F // WDR
    n_wo = Dh // WOR
    PA, PB = 0, 1

    a_k0, a_g0, a_u0, a_end = n_qa, n_qa + n_kv, n_qa + n_kv + n_g, n_qa + n_kv + n_g + UA
    b_v0, b_u0, b_d0, b_end = n_qb, n_qb + n_kv, n_qb + n_kv + UB, n_qb + n_kv + UB + n_d
    a_range = {"q": (0, a_k0), "k": (a_k0, a_g0), "g": (a_g0, a_u0), "u": (a_u0, a_end)}
    b_range = {"q": (0, b_v0), "v": (b_v0, b_u0), "u": (b_u0, b_d0), "d": (b_d0, b_end)}

    def wq_chunk(i, sem):
        rows = pl.ds(pl.multiple_of(_div(i, QS) * _SUBLANES, _SUBLANES), _SUBLANES)
        cols = pl.ds(pl.multiple_of(_mod(i, QS) * QC, _LANES), QC)
        return pltpu.make_async_copy(wq_hbm.at[rows, cols], wq_buf.at[rows, cols], sem)

    def kv_chunk(src, dst, s, sem):
        h, c = _div(s, C), _mod(s, C)
        return pltpu.make_async_copy(
            src.at[h, :, pl.ds(pl.multiple_of(Sk - W + c * KC, KC), KC)],
            dst.at[_mod(h, 2), :, pl.ds(pl.multiple_of(c * KC, KC), KC)], sem)

    def row_chunk(src, dst, first_row, nrows, sem):
        rows = pl.ds(pl.multiple_of(first_row, nrows), nrows)
        return pltpu.make_async_copy(src.at[rows], dst.at[rows], sem)

    def a_desc(kind, a):
        sem = sem_a.at[_mod(a, NSA)]
        if kind == "q":
            return wq_chunk(a + n_qb, sem)
        if kind == "k":
            return kv_chunk(k_hbm, kbuf, a - a_k0, sem)
        if kind == "g":
            return row_chunk(wg_hbm, wg_buf, (a - a_g0) * GR, GR, sem)
        return row_chunk(wu_hbm, wu_buf, (UB + a - a_u0) * GR, GR, sem)

    def b_desc(kind, b):
        sem = sem_b.at[_mod(b, NSB)]
        if kind == "q":
            return wq_chunk(b, sem)
        if kind == "v":
            return kv_chunk(v_hbm, vbuf, b - b_v0, sem)
        if kind == "u":
            return row_chunk(wu_hbm, wu_buf, (b - b_u0) * GR, GR, sem)
        return row_chunk(wd_hbm, wd_buf, (b - b_d0) * WDR, WDR, sem)

    def dispatch(desc, ranges, idx, lo, hi, action):
        for kind, (k_lo, k_hi) in ranges.items():
            if k_hi <= lo or k_lo >= hi or k_lo == k_hi:
                continue
            conds = []
            if k_lo > lo:
                conds.append(idx >= k_lo)
            if k_hi < hi:
                conds.append(idx < k_hi)
            if not conds:
                action(desc(kind, idx))
            else:
                cond = conds[0] if len(conds) == 1 else jnp.logical_and(conds[0], conds[1])
                pl.when(cond)(functools.partial(lambda kind: action(desc(kind, idx)), kind))

    def pump(t, lo, hi):
        dispatch(b_desc, b_range, t, lo, hi, lambda d: d.wait())
        dispatch(a_desc, a_range, t + KA, lo + KA, hi + KA, lambda d: d.start(priority=PA))
        dispatch(b_desc, b_range, t + VA, lo + VA, hi + VA, lambda d: d.start(priority=PB))
        dispatch(a_desc, a_range, t, lo, hi, lambda d: d.wait())

    def x_dma():
        return pltpu.make_async_copy(x_hbm, x_buf, sem_small.at[0])

    def wr_dma():
        return pltpu.make_async_copy(wr_hbm, wr_buf, sem_small.at[1])

    def wo_all(h):
        return pltpu.make_async_copy(wo_hbm.at[h], wo_buf.at[_mod(h, 2)], sem_wo.at[_mod(h, 2)])

    def wo_chunk(h, j):
        rows = pl.ds(pl.multiple_of(j * WOR, WOR), WOR)
        return pltpu.make_async_copy(wo_hbm.at[h, rows], wo_buf.at[_mod(h, 2), rows], sem_wo.at[_mod(h, 2)])

    def issue_wo(h, c):
        half = n_wo // 2

        @pl.when(c < half)
        def _():
            wo_chunk(h, 2 * c).start(priority=PB)

        @pl.when(jnp.logical_and(c >= C // 2, c < C // 2 + half))
        def _():
            wo_chunk(h, 2 * (c - C // 2) + 1).start(priority=PA)

    spread = VA // KA
    assert spread & (spread - 1) == 0 and KA * spread == VA and KA <= n_qa and VA <= n_qb

    def first(i, carry):
        @pl.when(_mod(i, spread) == 0)
        def _():
            a_desc("q", _div(i, spread)).start(priority=PA)

        b_desc("q", i).start(priority=PB)
        return carry

    lax.fori_loop(0, VA, first, 0)
    x_dma().start(priority=PA)
    wr_dma().start(priority=PA)

    scale = Dh ** -0.5

    def q_pair(p):
        cols = pl.ds(pl.multiple_of(p * (2 * Dh), _LANES), 2 * Dh)
        q2 = jnp.dot(xn_scr[...], wq_buf[:, cols], preferred_element_type=_F32).astype(_BF16)
        q_scr[2 * p] = q2[:, :Dh]
        q_scr[2 * p + 1] = q2[:, Dh:]

    def softmax():
        sc = s_scr[...]
        m = jnp.max(sc, axis=-1, keepdims=True)
        p = jnp.exp(sc - m)
        l_scr[...] = jnp.sum(p, axis=-1, keepdims=True)
        p_scr[...] = p.astype(_BF16)

    def pv_piece(h, j):
        cols = pl.ds(pl.multiple_of(j * PW, PW), PW)
        oacc_scr[...] += lax.dot_general(p_scr[:, cols], vbuf[_mod(h, 2), :, cols], (((1,), (1,)), ((), ())),
                                         preferred_element_type=_F32)

    def head_out(h):
        o = (oacc_scr[...] / l_scr[...]).astype(_BF16)
        wo_all(h).wait()
        return jnp.dot(o, wo_buf[_mod(h, 2)], preferred_element_type=_F32)

    t1 = a_k0 + C
    assert t1 >= n_qb

    def phase1(t, carry):
        pump(t, 0, t1)

        @pl.when(t >= a_k0)
        def _():
            issue_wo(0, t - a_k0)

        return carry

    lax.fori_loop(0, t1, phase1, 0)

    x_dma().wait()
    xn_scr[...] = _layernorm(x_buf[...].astype(_F32)).astype(_BF16)
    acc_scr[...] = jnp.zeros(acc_scr.shape, _F32)
    oacc_scr[...] = jnp.zeros(oacc_scr.shape, _F32)
    q_pair(0)
    s_scr[...] = jnp.dot(q_scr[0], kbuf[0], preferred_element_type=_F32) * scale
    softmax()

    def phase2(lo, hi, t, carry):
        s = t - a_k0
        h, c = _div(s, C), _mod(s, C)
        pump(t, lo, hi)
        issue_wo(h, c)

        @pl.when(_mod(c, CP) == CP // 2 - 1)
        def _():
            pv_piece(h - 1, _div(c, CP))

        @pl.when(c == C - 2)
        def _():
            acc_scr[...] += head_out(h - 1)
            oacc_scr[...] = jnp.zeros(oacc_scr.shape, _F32)

        @pl.when(jnp.logical_and(jnp.logical_and(c == CP + CP // 2 + 1, _mod(h, 2) == 1), h + 1 < H))
        def _():
            q_pair(_div(h + 1, 2))

        @pl.when(_mod(c, CP) == CP - 1)
        def _():
            cols = pl.ds(pl.multiple_of(_div(c, CP) * PW, PW), PW)
            s_scr[:, cols] = jnp.dot(q_scr[h], kbuf[_mod(h, 2), :, cols],
                                     preferred_element_type=_F32) * scale

        @pl.when(c == C - 1)
        def _():
            softmax()

        return carry

    t2 = a_g0
    t2m = min(a_g0 - KA, b_u0 - VA)
    lax.fori_loop(t1, t2m, functools.partial(phase2, t1, t2m), 0)
    lax.fori_loop(t2m, t2, functools.partial(phase2, t2m, t2), 0)

    t3 = a_end
    u_b_rows = UB * GR
    UA1 = UA - _LANES // GR
    u_mid = u_b_rows + UA1 * GR
    tau_u1 = max(LAG + UB, n_g) + 1
    tau_u2 = max(n_g + UA1, tau_u1 + 1)
    assert LAG < n_g and tau_u2 < t3 - t2

    def phase3(t, carry):
        pump(t, t2, t3)
        tau = t - t2

        @pl.when(jnp.logical_and(_mod(tau, CP) == CP // 2 - 1, tau < LAG))
        def _():
            pv_piece(H - 1, _div(tau, CP))

        @pl.when(tau == LAG)
        def _():
            hres = x_buf[...].astype(_F32) + acc_scr[...] + head_out(H - 1)
            hn = _layernorm(hres)
            hb = hn.astype(_BF16)
            wr_dma().wait()
            hf = hb.astype(_F32)
            rv = None
            for c in range(D // _LANES):
                tt = hf[:, c * _LANES:(c + 1) * _LANES] * wr_buf[c:c + 1, :].astype(_F32)
                rv = tt if rv is None else rv + tt
            r = jnp.sum(rv, axis=-1, keepdims=True)
            gate_scr[...] = jax.nn.sigmoid(r)
            hb_scr[...] = hb
            base_scr[...] = hres + (hn + hn * 0.0)

        @pl.when(tau == n_g)
        def _():
            g = jnp.dot(hb_scr[...], wg_buf[...], preferred_element_type=_F32)
            g_scr[...] = g * jax.nn.sigmoid(g)

        @pl.when(tau == tau_u1)
        def _():
            u_scr[...] = jnp.dot(hb_scr[:, :u_b_rows], wu_buf[pl.ds(0, u_b_rows), :],
                                 preferred_element_type=_F32)

        @pl.when(tau == tau_u2)
        def _():
            u_scr[...] += jnp.dot(hb_scr[:, u_b_rows:u_mid], wu_buf[pl.ds(u_b_rows, u_mid - u_b_rows), :],
                                  preferred_element_type=_F32)

        return carry

    lax.fori_loop(t2, t3, phase3, 0)

    u = u_scr[...] + jnp.dot(hb_scr[:, u_mid:], wu_buf[pl.ds(u_mid, D - u_mid), :],
                             preferred_element_type=_F32)
    a = (g_scr[...] * u).astype(_BF16)

    def wait_d(b, carry):
        b_desc("d", b).wait()
        return carry

    y = None
    row = 0
    done = t3
    assert done >= b_d0 and sum(DOWN) == F
    for rows in DOWN:
        need = b_d0 + (row + rows) // WDR
        if need > done:
            lax.fori_loop(done, need, wait_d, 0)
            done = need
        tt = jnp.dot(a[:, row:row + rows], wd_buf[pl.ds(row, rows), :], preferred_element_type=_F32)
        y = tt if y is None else y + tt
        row += rows
    assert done == b_end
    o_ref[...] = (base_scr[...] + y * gate_scr[...]).astype(o_ref.dtype)


def _build(KA=12, VA=48, NP=4, UA=24, WOR=24, WDR=32, DOWN=(640, 384, 256, 128, 128), interpret=False):
    def fn(A_x, A_k_cache, A_v_cache, A_wq, A_wo, B_x, B_w_r, B_w_gate, B_w_up, B_w_down):
        B, Sq, D = A_x.shape
        _, H, Sk, Dh = A_k_cache.shape
        F = B_w_gate.shape[1]
        W = min(4096, max(256, Sk // 4))
        assert B == 1 and Sq == 1

        kt = jnp.swapaxes(A_k_cache, 2, 3).reshape(H, Dh, Sk)
        vt = jnp.swapaxes(A_v_cache, 2, 3).reshape(H, Dh, Sk)
        x2 = A_x.reshape(1, D)
        wr2 = B_w_r.reshape(D // _LANES, _LANES)
        wo3 = A_wo.reshape(H, Dh, D)

        kern = functools.partial(_kernel, H=H, Dh=Dh, Sk=Sk, W=W, D=D, F=F, KA=KA, VA=VA, NP=NP,
                                 UA=UA, WOR=WOR, WDR=WDR, DOWN=DOWN)
        any_spec = pl.BlockSpec(memory_space=pl.ANY)
        out = pl.pallas_call(
            kern,
            out_shape=jax.ShapeDtypeStruct((1, D), A_x.dtype),
            in_specs=[any_spec] * 9,
            out_specs=pl.BlockSpec(memory_space=pltpu.VMEM),
            scratch_shapes=[
                pltpu.VMEM((1, D), _BF16),
                pltpu.VMEM((D // _LANES, _LANES), _BF16),
                pltpu.VMEM((2, Dh, W), _BF16),
                pltpu.VMEM((2, Dh, W), _BF16),
                pltpu.VMEM((D, H * Dh), _BF16),
                pltpu.VMEM((2, Dh, D), _BF16),
                pltpu.VMEM((D, F), _BF16),
                pltpu.VMEM((D, F), _BF16),
                pltpu.VMEM((F, D), _BF16),
                pltpu.VMEM((1, D), _BF16),
                pltpu.VMEM((H, 1, Dh), _BF16),
                pltpu.VMEM((1, W), _F32),
                pltpu.VMEM((1, W), _BF16),
                pltpu.VMEM((1, 1), _F32),
                pltpu.VMEM((1, Dh), _F32),
                pltpu.VMEM((1, D), _F32),
                pltpu.VMEM((1, D), _BF16),
                pltpu.VMEM((1, D), _F32),
                pltpu.VMEM((1, 1), _F32),
                pltpu.VMEM((1, F), _F32),
                pltpu.VMEM((1, F), _F32),
                pltpu.SemaphoreType.DMA((2,)),
                pltpu.SemaphoreType.DMA((1 << KA.bit_length(),)),
                pltpu.SemaphoreType.DMA((1 << VA.bit_length(),)),
                pltpu.SemaphoreType.DMA((2,)),
            ],
            compiler_params=pltpu.CompilerParams(vmem_limit_bytes=64 * 1024 * 1024,
                                                 disable_bounds_checks=True,
                                                 disable_semaphore_checks=True),
            interpret=interpret,
        )(x2, wr2, kt, vt, A_wq, wo3, B_w_gate, B_w_up, B_w_down)
        return out.reshape(B, Sq, D)
    return fn


@jax.jit
def pallas_sequential_preLN__sliding_block_cached__moe_arch_mod__decode_kernel(
    A_x: jax.Array,
    A_k_cache: jax.Array,
    A_v_cache: jax.Array,
    A_wq: jax.Array,
    A_wo: jax.Array,
    B_x: jax.Array,
    B_w_r: jax.Array,
    B_w_gate: jax.Array,
    B_w_up: jax.Array,
    B_w_down: jax.Array,
):
    return _build()(A_x, A_k_cache, A_v_cache, A_wq, A_wo, B_x, B_w_r, B_w_gate, B_w_up, B_w_down)
```

```python
import functools

import jax
import jax.numpy as jnp
from jax import lax
import jax.experimental.pallas as pl
import jax.experimental.pallas.tpu as pltpu

_F32 = jnp.float32
_BF16 = jnp.bfloat16
_LN_EPS = 1e-5
_LANES = 128
_SUBLANES = 8


def _layernorm(x):
    m = jnp.mean(x, axis=-1, keepdims=True)
    c = x - m
    v = jnp.mean(c * c, axis=-1, keepdims=True)
    return c / jnp.sqrt(v + _LN_EPS)


def _log2(n):
    assert n > 0 and n & (n - 1) == 0, n
    return n.bit_length() - 1


def _div(x, n):
    if isinstance(x, int):
        return x // n
    if n & (n - 1) == 0:
        return lax.shift_right_logical(x, _log2(n))
    return lax.div(x, jnp.int32(n))


def _mod(x, n):
    if isinstance(x, int) or n & (n - 1) == 0:
        return x % n if isinstance(x, int) else x & (n - 1)
    return lax.rem(x, jnp.int32(n))


def _kernel(x_hbm, wr_hbm, k_hbm, v_hbm, wq_hbm, wo_hbm, wg_hbm, wu_hbm, wd_hbm,
            o_ref,
            x_buf, wr_buf, kbuf, vbuf, wq_buf, wo_buf, wg_buf, wu_buf, wd_buf,
            xn_scr, q_scr, s_scr, p_scr, l_scr, oacc_scr, acc_scr,
            hb_scr, base_scr, gate_scr, g_scr, u_scr,
            sem_small, sem_a, sem_b, sem_wo,
            *, H, Dh, Sk, W, D, F, KA, VA, NP, UA, WOR, WDR, DOWN, QC):
    KC = _LANES
    C = W // KC
    CP = C // NP
    PW = W // NP
    NSA = 1 << KA.bit_length()
    NSB = 1 << VA.bit_length()
    LAG = C - CP // 2
    QG = wq_hbm.shape[1]
    QS = (H * Dh) // QC
    n_q = QG * QS
    n_qa = (n_q - LAG) // 2
    n_qb = n_q - n_qa
    assert n_qb - n_qa == LAG
    GR = Dh * KC // F
    n_kv = H * C
    n_g = D // GR
    UB = n_g - UA
    n_d = F // WDR
    n_wo = Dh // WOR
    PA, PB = 0, 1

    a_k0, a_g0, a_u0, a_end = n_qa, n_qa + n_kv, n_qa + n_kv + n_g, n_qa + n_kv + n_g + UA
    b_v0, b_u0, b_d0, b_end = n_qb, n_qb + n_kv, n_qb + n_kv + UB, n_qb + n_kv + UB + n_d
    a_range = {"q": (0, a_k0), "k": (a_k0, a_g0), "g": (a_g0, a_u0), "u": (a_u0, a_end)}
    b_range = {"q": (0, b_v0), "v": (b_v0, b_u0), "u": (b_u0, b_d0), "d": (b_d0, b_end)}

    def wq_chunk(i, sem):
        g = _div(i, QS)
        cols = pl.ds(pl.multiple_of(_mod(i, QS) * QC, _LANES), QC)
        return pltpu.make_async_copy(wq_hbm.at[:, g, :, cols], wq_buf.at[:, g, :, cols], sem)

    def kv_chunk(src, dst, s, sem):
        h, c = _div(s, C), _mod(s, C)
        return pltpu.make_async_copy(
            src.at[h, :, pl.ds(pl.multiple_of(Sk - W + c * KC, KC), KC)],
            dst.at[_mod(h, 2), :, pl.ds(pl.multiple_of(c * KC, KC), KC)], sem)

    def row_chunk(src, dst, first_row, nrows, sem):
        rows = pl.ds(pl.multiple_of(first_row, nrows), nrows)
        return pltpu.make_async_copy(src.at[rows], dst.at[rows], sem)

    def a_desc(kind, a):
        sem = sem_a.at[_mod(a, NSA)]
        if kind == "q":
            return wq_chunk(a + n_qb, sem)
        if kind == "k":
            return kv_chunk(k_hbm, kbuf, a - a_k0, sem)
        if kind == "g":
            return row_chunk(wg_hbm, wg_buf, (a - a_g0) * GR, GR, sem)
        return row_chunk(wu_hbm, wu_buf, (UB + a - a_u0) * GR, GR, sem)

    def b_desc(kind, b):
        sem = sem_b.at[_mod(b, NSB)]
        if kind == "q":
            return wq_chunk(b, sem)
        if kind == "v":
            return kv_chunk(v_hbm, vbuf, b - b_v0, sem)
        if kind == "u":
            return row_chunk(wu_hbm, wu_buf, (b - b_u0) * GR, GR, sem)
        return row_chunk(wd_hbm, wd_buf, (b - b_d0) * WDR, WDR, sem)

    def dispatch(desc, ranges, idx, lo, hi, action):
        for kind, (k_lo, k_hi) in ranges.items():
            if k_hi <= lo or k_lo >= hi or k_lo == k_hi:
                continue
            conds = []
            if k_lo > lo:
                conds.append(idx >= k_lo)
            if k_hi < hi:
                conds.append(idx < k_hi)
            if not conds:
                action(desc(kind, idx))
            else:
                cond = conds[0] if len(conds) == 1 else jnp.logical_and(conds[0], conds[1])
                pl.when(cond)(functools.partial(lambda kind: action(desc(kind, idx)), kind))

    def pump(t, lo, hi):
        dispatch(b_desc, b_range, t, lo, hi, lambda d: d.wait())
        dispatch(a_desc, a_range, t + KA, lo + KA, hi + KA, lambda d: d.start(priority=PA))
        dispatch(b_desc, b_range, t + VA, lo + VA, hi + VA, lambda d: d.start(priority=PB))
        dispatch(a_desc, a_range, t, lo, hi, lambda d: d.wait())

    def x_dma():
        return pltpu.make_async_copy(x_hbm, x_buf, sem_small.at[0])

    def wr_dma():
        return pltpu.make_async_copy(wr_hbm, wr_buf, sem_small.at[1])

    def wo_all(h):
        return pltpu.make_async_copy(wo_hbm.at[h], wo_buf.at[_mod(h, 2)], sem_wo.at[_mod(h, 2)])

    def wo_chunk(h, j):
        rows = pl.ds(pl.multiple_of(j * WOR, WOR), WOR)
        return pltpu.make_async_copy(wo_hbm.at[h, rows], wo_buf.at[_mod(h, 2), rows], sem_wo.at[_mod(h, 2)])

    def issue_wo(h, c):
        half = n_wo // 2

        @pl.when(c < half)
        def _():
            wo_chunk(h, 2 * c).start(priority=PB)

        @pl.when(jnp.logical_and(c >= C // 2, c < C // 2 + half))
        def _():
            wo_chunk(h, 2 * (c - C // 2) + 1).start(priority=PA)

    spread = VA // KA
    assert spread & (spread - 1) == 0 and KA * spread == VA and KA <= n_qa and VA <= n_qb

    def first(i, carry):
        @pl.when(_mod(i, spread) == 0)
        def _():
            a_desc("q", _div(i, spread)).start(priority=PA)

        b_desc("q", i).start(priority=PB)
        return carry

    lax.fori_loop(0, VA, first, 0)
    x_dma().start(priority=PA)
    wr_dma().start(priority=PA)

    scale = Dh ** -0.5

    def q_pair(p):
        cols = pl.ds(pl.multiple_of(p * (2 * Dh), _LANES), 2 * Dh)
        w = wq_buf[:, :, :, cols].reshape(D, 2 * Dh)
        q2 = jnp.dot(xn_scr[...], w, preferred_element_type=_F32).astype(_BF16)
        q_scr[2 * p] = q2[:, :Dh]
        q_scr[2 * p + 1] = q2[:, Dh:]

    def softmax():
        sc = s_scr[...]
        m = jnp.max(sc, axis=-1, keepdims=True)
        p = jnp.exp(sc - m)
        l_scr[...] = jnp.sum(p, axis=-1, keepdims=True)
        p_scr[...] = p.astype(_BF16)

    def pv_piece(h, j):
        cols = pl.ds(pl.multiple_of(j * PW, PW), PW)
        oacc_scr[...] += lax.dot_general(p_scr[:, cols], vbuf[_mod(h, 2), :, cols], (((1,), (1,)), ((), ())),
                                         preferred_element_type=_F32)

    def head_out(h):
        o = (oacc_scr[...] / l_scr[...]).astype(_BF16)
        wo_all(h).wait()
        return jnp.dot(o, wo_buf[_mod(h, 2)], preferred_element_type=_F32)

    t1 = a_k0 + C
    assert t1 >= n_qb

    def phase1(t, carry):
        pump(t, 0, t1)

        @pl.when(t >= a_k0)
        def _():
            issue_wo(0, t - a_k0)

        return carry

    lax.fori_loop(0, t1, phase1, 0)

    x_dma().wait()
    xn_scr[...] = _layernorm(x_buf[...].astype(_F32)).astype(_BF16)
    acc_scr[...] = jnp.zeros(acc_scr.shape, _F32)
    oacc_scr[...] = jnp.zeros(oacc_scr.shape, _F32)
    q_pair(0)
    s_scr[...] = jnp.dot(q_scr[0], kbuf[0], preferred_element_type=_F32) * scale
    softmax()

    def phase2(lo, hi, t, carry):
        s = t - a_k0
        h, c = _div(s, C), _mod(s, C)
        pump(t, lo, hi)
        issue_wo(h, c)

        @pl.when(_mod(c, CP) == CP // 2 - 1)
        def _():
            pv_piece(h - 1, _div(c, CP))

        @pl.when(c == C - 2)
        def _():
            acc_scr[...] += head_out(h - 1)
            oacc_scr[...] = jnp.zeros(oacc_scr.shape, _F32)

        @pl.when(jnp.logical_and(jnp.logical_and(c == CP + CP // 2 + 1, _mod(h, 2) == 1), h + 1 < H))
        def _():
            q_pair(_div(h + 1, 2))

        @pl.when(_mod(c, CP) == CP - 1)
        def _():
            cols = pl.ds(pl.multiple_of(_div(c, CP) * PW, PW), PW)
            s_scr[:, cols] = jnp.dot(q_scr[h], kbuf[_mod(h, 2), :, cols],
                                     preferred_element_type=_F32) * scale

        @pl.when(c == C - 1)
        def _():
            softmax()

        return carry

    t2 = a_g0
    t2m = min(a_g0 - KA, b_u0 - VA)
    lax.fori_loop(t1, t2m, functools.partial(phase2, t1, t2m), 0)
    lax.fori_loop(t2m, t2, functools.partial(phase2, t2m, t2), 0)

    t3 = a_end
    u_b_rows = UB * GR
    UA1 = UA - _LANES // GR
    u_mid = u_b_rows + UA1 * GR
    tau_u1 = max(LAG + UB, n_g) + 1
    tau_u2 = max(n_g + UA1, tau_u1 + 1)
    assert LAG < n_g and tau_u2 < t3 - t2

    def phase3(t, carry):
        pump(t, t2, t3)
        tau = t - t2

        @pl.when(jnp.logical_and(_mod(tau, CP) == CP // 2 - 1, tau < LAG))
        def _():
            pv_piece(H - 1, _div(tau, CP))

        @pl.when(tau == LAG)
        def _():
            hres = x_buf[...].astype(_F32) + acc_scr[...] + head_out(H - 1)
            hn = _layernorm(hres)
            hb = hn.astype(_BF16)
            wr_dma().wait()
            hf = hb.astype(_F32)
            rv = None
            for c in range(D // _LANES):
                tt = hf[:, c * _LANES:(c + 1) * _LANES] * wr_buf[c:c + 1, :].astype(_F32)
                rv = tt if rv is None else rv + tt
            r = jnp.sum(rv, axis=-1, keepdims=True)
            gate_scr[...] = jax.nn.sigmoid(r)
            hb_scr[...] = hb
            base_scr[...] = hres + (hn + hn * 0.0)

        @pl.when(tau == n_g)
        def _():
            g = jnp.dot(hb_scr[...], wg_buf[...], preferred_element_type=_F32)
            g_scr[...] = g * jax.nn.sigmoid(g)

        @pl.when(tau == tau_u1)
        def _():
            u_scr[...] = jnp.dot(hb_scr[:, :u_b_rows], wu_buf[pl.ds(0, u_b_rows), :],
                                 preferred_element_type=_F32)

        @pl.when(tau == tau_u2)
        def _():
            u_scr[...] += jnp.dot(hb_scr[:, u_b_rows:u_mid], wu_buf[pl.ds(u_b_rows, u_mid - u_b_rows), :],
                                  preferred_element_type=_F32)

        return carry

    lax.fori_loop(t2, t3, phase3, 0)

    u = u_scr[...] + jnp.dot(hb_scr[:, u_mid:], wu_buf[pl.ds(u_mid, D - u_mid), :],
                             preferred_element_type=_F32)
    a = (g_scr[...] * u).astype(_BF16)

    def wait_d(b, carry):
        b_desc("d", b).wait()
        return carry

    y = None
    row = 0
    done = t3
    assert done >= b_d0 and sum(DOWN) == F
    for rows in DOWN:
        need = b_d0 + (row + rows) // WDR
        if need > done:
            lax.fori_loop(done, need, wait_d, 0)
            done = need
        tt = jnp.dot(a[:, row:row + rows], wd_buf[pl.ds(row, rows), :], preferred_element_type=_F32)
        y = tt if y is None else y + tt
        row += rows
    assert done == b_end
    o_ref[...] = (base_scr[...] + y * gate_scr[...]).astype(o_ref.dtype)


def _build(KA=12, VA=48, NP=4, UA=24, WOR=24, WDR=32, DOWN=(640, 384, 256, 128, 128), QB=5, QC=384,
           interpret=False):
    def fn(A_x, A_k_cache, A_v_cache, A_wq, A_wo, B_x, B_w_r, B_w_gate, B_w_up, B_w_down):
        B, Sq, D = A_x.shape
        _, H, Sk, Dh = A_k_cache.shape
        F = B_w_gate.shape[1]
        W = min(4096, max(256, Sk // 4))
        assert B == 1 and Sq == 1

        kt = jnp.swapaxes(A_k_cache, 2, 3).reshape(H, Dh, Sk)
        vt = jnp.swapaxes(A_v_cache, 2, 3).reshape(H, Dh, Sk)
        x2 = A_x.reshape(1, D)
        wr2 = B_w_r.reshape(D // _LANES, _LANES)
        wo3 = A_wo.reshape(H, Dh, D)
        wq4 = A_wq.reshape(QB, D // (QB * _SUBLANES), _SUBLANES, H * Dh)

        kern = functools.partial(_kernel, H=H, Dh=Dh, Sk=Sk, W=W, D=D, F=F, KA=KA, VA=VA, NP=NP,
                                 UA=UA, WOR=WOR, WDR=WDR, DOWN=DOWN, QC=QC)
        any_spec = pl.BlockSpec(memory_space=pl.ANY)
        out = pl.pallas_call(
            kern,
            out_shape=jax.ShapeDtypeStruct((1, D), A_x.dtype),
            in_specs=[any_spec] * 9,
            out_specs=pl.BlockSpec(memory_space=pltpu.VMEM),
            scratch_shapes=[
                pltpu.VMEM((1, D), _BF16),
                pltpu.VMEM((D // _LANES, _LANES), _BF16),
                pltpu.VMEM((2, Dh, W), _BF16),
                pltpu.VMEM((2, Dh, W), _BF16),
                pltpu.VMEM((QB, D // (QB * _SUBLANES), _SUBLANES, H * Dh), _BF16),
                pltpu.VMEM((2, Dh, D), _BF16),
                pltpu.VMEM((D, F), _BF16),
                pltpu.VMEM((D, F), _BF16),
                pltpu.VMEM((F, D), _BF16),
                pltpu.VMEM((1, D), _BF16),
                pltpu.VMEM((H, 1, Dh), _BF16),
                pltpu.VMEM((1, W), _F32),
                pltpu.VMEM((1, W), _BF16),
                pltpu.VMEM((1, 1), _F32),
                pltpu.VMEM((1, Dh), _F32),
                pltpu.VMEM((1, D), _F32),
                pltpu.VMEM((1, D), _BF16),
                pltpu.VMEM((1, D), _F32),
                pltpu.VMEM((1, 1), _F32),
                pltpu.VMEM((1, F), _F32),
                pltpu.VMEM((1, F), _F32),
                pltpu.SemaphoreType.DMA((2,)),
                pltpu.SemaphoreType.DMA((1 << KA.bit_length(),)),
                pltpu.SemaphoreType.DMA((1 << VA.bit_length(),)),
                pltpu.SemaphoreType.DMA((2,)),
            ],
            compiler_params=pltpu.CompilerParams(vmem_limit_bytes=64 * 1024 * 1024,
                                                 disable_bounds_checks=True,
                                                 disable_semaphore_checks=True),
            interpret=interpret,
        )(x2, wr2, kt, vt, wq4, wo3, B_w_gate, B_w_up, B_w_down)
        return out.reshape(B, Sq, D)
    return fn


@jax.jit
def pallas_sequential_preLN__sliding_block_cached__moe_arch_mod__decode_kernel(
    A_x: jax.Array,
    A_k_cache: jax.Array,
    A_v_cache: jax.Array,
    A_wq: jax.Array,
    A_wo: jax.Array,
    B_x: jax.Array,
    B_w_r: jax.Array,
    B_w_gate: jax.Array,
    B_w_up: jax.Array,
    B_w_down: jax.Array,
):
    return _build()(A_x, A_k_cache, A_v_cache, A_wq, A_wo, B_x, B_w_r, B_w_gate, B_w_up, B_w_down)
```
